```python
import os as _os
_os.environ.setdefault("JAX_PLATFORMS", "cpu")
import jax
import jax.numpy as jnp

def _softmax(x, axis=-1):
    return jax.nn.softmax(x, axis=axis)
def _gelu(x):
    return jax.nn.gelu(x, approximate=True)
def _silu(x):
    return jax.nn.silu(x)
def _sigmoid(x):
    return jax.nn.sigmoid(x)
def _layernorm(x, axis=-1, eps=1e-5):
    m = jnp.mean(x, axis=axis, keepdims=True)
    v = jnp.var(x, axis=axis, keepdims=True)
    return (x - m) / jnp.sqrt(v + eps)
def _scatter_add(tgt, idx, src, axis=0):
    return tgt.at[idx].add(src)
def _segment_sum(src, seg, n):
    return jax.ops.segment_sum(src, seg, n)
class _Rng:
    def __init__(self, key):
        self._k = key
    def _next(self):
        self._k, sub = jax.random.split(self._k)
        return sub
    def normal(self, shape):
        return jax.random.normal(self._next(), shape, dtype=jnp.bfloat16)
    def randint(self, lo, hi, shape):
        return jax.random.randint(self._next(), shape, lo, hi, dtype=jnp.int32)
    def uniform(self, shape, lo=0.0, hi=1.0):
        return jax.random.uniform(self._next(), shape, jnp.bfloat16, lo, hi)
    def permutation(self, n):
        return jax.random.permutation(self._next(), n)


kernel_name = 'parallel_sum__softmax_full_mha__glu_gated_swiglu__prompt'

def setup_inputs():
    _rng = _Rng(jax.random.key(int.from_bytes(__import__("os").urandom(4), "little")))
    _w = (lambda a: (lambda t: t.astype(jnp.bfloat16) if jnp.issubdtype(t.dtype, jnp.floating) else t)(jnp.asarray(a)))
    def _A_setup():
        B, S, D = 1, 2048, 448
        return {
            "x": _w((lambda *s: _rng.normal(s) * 0.05)(B, S, D)),
            "wqkv": _w((lambda *s: _rng.normal(s) * 0.05)(D, 3 * D)),
            "wo": _w((lambda *s: _rng.normal(s) * 0.05)(D, D)),
        }
    _A_in = _A_setup()

    def _B_setup():
        B, S, D, F = 1, 2048, 448, 1792
        return {
            "x": _w((lambda *s: _rng.normal(s) * 0.05)(B, S, D)),
            "w1": _w((lambda *s: _rng.normal(s) * 0.05)(D, F) * (2.0 / D) ** 0.5),
            "w3": _w((lambda *s: _rng.normal(s) * 0.05)(D, F) * (2.0 / D) ** 0.5),
            "w2": _w((lambda *s: _rng.normal(s) * 0.05)(F, D) * (2.0 / F) ** 0.5),
        }
    _B_in = _B_setup()

    return {
        "A_x": _A_in["x"],
        "A_wqkv": _A_in["wqkv"],
        "A_wo": _A_in["wo"],
        "B_x": _B_in["x"],
        "B_w1": _B_in["w1"],
        "B_w3": _B_in["w3"],
        "B_w2": _B_in["w2"],
    }

def reference(A_x, A_wqkv, A_wo, B_x, B_w1, B_w3, B_w2):
    def _A_ref(x, wqkv, wo):
        B, S, D = x.shape
        H = 16; Dh = D // H
        qkv = (lambda x, *d: x.transpose(*d))((x @ wqkv).reshape(B, S, 3, H, Dh), 2, 0, 3, 1, 4)
        q, k, v = qkv[0], qkv[1], qkv[2]
        scale = Dh ** -0.5
        scores = jnp.einsum("bhqd,bhkd->bhqk", q, k) * scale
        p = _softmax(scores, axis=-1)
        o = jnp.einsum("bhqk,bhkd->bhqd", p, v)
        return (lambda x, *d: x.transpose(*d))(o, 0, 2, 1, 3).reshape(B, S, D) @ wo

    def _B_ref(x, w1, w3, w2):
        gate = jnp.einsum("bsd,df->bsf", x, w1)
        up = jnp.einsum("bsd,df->bsf", x, w3)
        h = _silu(gate) * up
        out = jnp.einsum("bsf,fd->bsd", h, w2)
        return out

    x = A_x
    xn = _layernorm(x, axis=-1)
    return x + _A_ref(xn, A_wqkv, A_wo) + _B_ref(xn, B_w1, B_w3, B_w2)
```

```python
import math

import jax
import jax.numpy as jnp
import jax.experimental.pallas as pl
import jax.experimental.pallas.tpu as pltpu

S = 2048
D = 448
H = 16
DH = D // H
F = 1792
G = 4
GW = 4 * DH
HP = 32
M = 512
C = 256
TB = 512
FC = 256
NI = (S // M) * H
NC = S // C
EPS = 1e-5
QSCALE = (DH ** -0.5) * math.log2(math.e)

_NT = (((1,), (1,)), ((), ()))
_TN = (((0,), (0,)), ((), ()))
f32 = jnp.float32
bf16 = jnp.bfloat16


def _kernel(x_hbm, wqkv_hbm, wo_hbm, w1_hbm, w3_hbm, w2_hbm, out_hbm,
            x_v, wqkv_v, wo_v, w1_v, w3_v, w2_v,
            xn_v, wqv_v, wk_v, wop_v, t32,
            k_ref, qm_ref, vt_ref, s_a, s_b, m_a, m_b, ot_ref, h_ref, out_v,
            in_sems, out_sems):
    nxb = S // TB
    x_copies = [
        pltpu.make_async_copy(x_hbm.at[pl.ds(b * TB, TB), :],
                              x_v.at[pl.ds(b * TB, TB), :], in_sems.at[b])
        for b in range(nxb)
    ]
    cp_wqkv = pltpu.make_async_copy(wqkv_hbm, wqkv_v, in_sems.at[nxb])
    cp_wo = pltpu.make_async_copy(wo_hbm, wo_v, in_sems.at[nxb + 1])
    cp_w1 = pltpu.make_async_copy(w1_hbm, w1_v, in_sems.at[nxb + 2])
    cp_w3 = pltpu.make_async_copy(w3_hbm, w3_v, in_sems.at[nxb + 3])
    cp_w2 = pltpu.make_async_copy(w2_hbm, w2_v, in_sems.at[nxb + 4])
    cp_wqkv.start()
    for cp in x_copies:
        cp.start()
    cp_wo.start()
    cp_w1.start()
    cp_w3.start()
    cp_w2.start()

    cp_wqkv.wait()
    wt = wqkv_v[...].T
    wqv_v[0:D, :] = wt[0:D]
    z16 = jnp.zeros((128 - GW, D), bf16)
    for g in range(G):
        wk_v[128 * g:128 * g + GW, :] = wt[D + GW * g:D + GW * (g + 1)]
        wk_v[128 * g + GW:128 * (g + 1), :] = z16
    t32[...] = wt[2 * D:3 * D].astype(f32)
    z4 = jnp.zeros((HP - DH, D), f32)
    for h in range(H):
        wqv_v[D + HP * h:D + HP * (h + 1), :] = jnp.concatenate(
            [t32[DH * h:DH * (h + 1), :], z4], axis=0).astype(bf16)

    row128 = jax.lax.broadcasted_iota(jnp.int32, (128, TB), 0)
    row32 = jax.lax.broadcasted_iota(jnp.int32, (HP, TB), 0)
    for b in range(nxb):
        x_copies[b].wait()
        rows = slice(b * TB, (b + 1) * TB)
        x = x_v[rows, :].astype(f32)
        mu = jnp.mean(x, axis=-1, keepdims=True)
        xc = x - mu
        var = jnp.mean(xc * xc, axis=-1, keepdims=True)
        xn = (xc * jax.lax.rsqrt(var + EPS)).astype(bf16)
        xn_v[rows, :] = xn
        k = jax.lax.dot_general(xn, wk_v[...], _NT, preferred_element_type=f32)
        for g in range(G):
            k_ref[g, rows, :] = k[:, 128 * g:128 * (g + 1)].astype(bf16)
        qv = jax.lax.dot_general(wqv_v[...], xn, _NT, preferred_element_type=f32)
        zq = jnp.zeros((128 - GW, TB), f32)
        for g in range(G):
            qg = jnp.concatenate([qv[GW * g:GW * (g + 1)] * QSCALE, zq], axis=0)
            for j in range(4):
                sel = (row128 >= DH * j) & (row128 < DH * (j + 1))
                qm_ref[4 * g + j, :, rows] = jnp.where(sel, qg, 0.0).astype(bf16)
        for h in range(H):
            v = qv[D + HP * h:D + HP * (h + 1)]
            vt_ref[h, :, rows] = jnp.where(row32 == DH, 1.0, v).astype(bf16)

    def idx(it):
        it = jnp.minimum(it, NI - 1)
        h = jax.lax.rem(it, H)
        qb = jax.lax.div(it, H)
        return h, pl.multiple_of(qb * M, M)

    def qk_chunk(h, q0, c, s_out, mrun):
        g = h // 4
        qm = qm_ref[h, :, pl.ds(q0, M)]
        s = jnp.dot(k_ref[g, c * C:(c + 1) * C, :], qm, preferred_element_type=f32)
        s_out[c * C:(c + 1) * C, :] = s
        mc = jnp.max(s.reshape(C // 8, 8, M), axis=0)
        return mc if mrun is None else jnp.maximum(mrun, mc)

    def pv_chunk(h, c, s_in, m, o):
        p = jnp.exp2(s_in[c * C:(c + 1) * C, :] - m).astype(bf16)
        oc = jnp.dot(vt_ref[h, :, c * C:(c + 1) * C], p, preferred_element_type=f32)
        return oc if o is None else o + oc

    def step(cur, s_cur, m_cur, s_nxt, m_nxt):
        h, q0 = idx(cur)
        h2, q2 = idx(cur + 1)
        m = m_cur[...]
        mrun = None
        o = None
        for c in range(NC):
            mrun = qk_chunk(h2, q2, c, s_nxt, mrun)
            o = pv_chunk(h, c, s_cur, m, o)
        m_nxt[...] = jnp.max(mrun, axis=0, keepdims=True)
        inv = 1.0 / o[DH:DH + 1, :]
        ot_ref[h, :, pl.ds(q0, M)] = (o * inv).astype(bf16)

    mrun = None
    for c in range(NC):
        mrun = qk_chunk(0, 0, c, s_a, mrun)
    m_a[...] = jnp.max(mrun, axis=0, keepdims=True)

    def attn_body(i, carry):
        step(2 * i, s_a, m_a, s_b, m_b)
        step(2 * i + 1, s_b, m_b, s_a, m_a)
        return carry

    jax.lax.fori_loop(0, NI // 2, attn_body, 0)

    cp_wo.wait()
    cp_w1.wait()
    cp_w3.wait()
    cp_w2.wait()
    t32[...] = wo_v[...].astype(f32)
    for h in range(H):
        wop_v[HP * h:HP * (h + 1), :] = jnp.concatenate(
            [t32[DH * h:DH * (h + 1), :], z4], axis=0).astype(bf16)

    def out_copy(b):
        r0 = pl.multiple_of(b * TB, TB)
        return pltpu.make_async_copy(out_v.at[pl.ds(r0, TB), :],
                                     out_hbm.at[pl.ds(r0, TB), :], out_sems.at[b])

    def ffn_body(b, carry):
        r0 = pl.multiple_of(b * TB, TB)
        xn = xn_v[pl.ds(r0, TB), :]
        for c in range(F // FC):
            cols = slice(c * FC, (c + 1) * FC)
            gate = jnp.dot(xn, w1_v[:, cols], preferred_element_type=f32)
            up = jnp.dot(xn, w3_v[:, cols], preferred_element_type=f32)
            h_ref[:, cols] = (gate * jax.nn.sigmoid(gate) * up).astype(bf16)
        ot = ot_ref[:, :, pl.ds(r0, TB)].reshape(H * HP, TB)
        acc = jax.lax.dot_general(ot, wop_v[...], _TN, preferred_element_type=f32)
        acc = acc + jnp.dot(h_ref[...], w2_v[...], preferred_element_type=f32)
        acc = acc + x_v[pl.ds(r0, TB), :].astype(f32)
        out_v[pl.ds(r0, TB), :] = acc.astype(bf16)
        out_copy(b).start()
        return carry

    jax.lax.fori_loop(0, nxb, ffn_body, 0)
    for b in range(nxb):
        out_copy(b).wait()


@jax.jit
def pallas_parallel_sum__softmax_full_mha__glu_gated_swiglu__prompt_kernel(
    A_x: jax.Array,
    A_wqkv: jax.Array,
    A_wo: jax.Array,
    B_x: jax.Array,
    B_w1: jax.Array,
    B_w3: jax.Array,
    B_w2: jax.Array,
):
    del B_x
    x = A_x.reshape(S, D)
    any_spec = pl.BlockSpec(memory_space=pl.ANY)
    out = pl.pallas_call(
        _kernel,
        out_shape=jax.ShapeDtypeStruct((S, D), bf16),
        in_specs=[any_spec] * 6,
        out_specs=any_spec,
        scratch_shapes=[
            pltpu.VMEM((S, D), bf16),
            pltpu.VMEM((D, 3 * D), bf16),
            pltpu.VMEM((D, D), bf16),
            pltpu.VMEM((D, F), bf16),
            pltpu.VMEM((D, F), bf16),
            pltpu.VMEM((F, D), bf16),
            pltpu.VMEM((S, D), bf16),
            pltpu.VMEM((D + H * HP, D), bf16),
            pltpu.VMEM((G * 128, D), bf16),
            pltpu.VMEM((H * HP, D), bf16),
            pltpu.VMEM((D, D), f32),
            pltpu.VMEM((G, S, 128), bf16),
            pltpu.VMEM((H, 128, S), bf16),
            pltpu.VMEM((H, HP, S), bf16),
            pltpu.VMEM((S, M), f32),
            pltpu.VMEM((S, M), f32),
            pltpu.VMEM((1, M), f32),
            pltpu.VMEM((1, M), f32),
            pltpu.VMEM((H, HP, S), bf16),
            pltpu.VMEM((TB, F), bf16),
            pltpu.VMEM((S, D), bf16),
            pltpu.SemaphoreType.DMA((S // TB + 5,)),
            pltpu.SemaphoreType.DMA((S // TB,)),
        ],
        compiler_params=pltpu.CompilerParams(vmem_limit_bytes=100 * 1024 * 1024),
    )(x, A_wqkv, A_wo, B_w1, B_w3, B_w2)
    return out.reshape(1, S, D)
```

```python
import math

import jax
import jax.numpy as jnp
import jax.experimental.pallas as pl
import jax.experimental.pallas.tpu as pltpu

S = 2048
D = 448
H = 16
DH = D // H
F = 1792
G = 4
HP = 32
QT = 128
W = 4 * QT
BQ = 256
C = 128
LAG = 2
TB = 512
FC = 128
NTAIL = 4
NC = S // C
EPS = 1e-5
QSCALE = (DH ** -0.5) * math.log2(math.e)

_NT = (((1,), (1,)), ((), ()))
f32 = jnp.float32
bf16 = jnp.bfloat16


def _kernel(x_hbm, wqkv_hbm, wo_hbm, w1_hbm, w3_hbm, w2_hbm, out_hbm,
            x_v, wqkv_v, wo_v, w1_v, w3_v, w2_v,
            xn_v, wqv_v, wk_v, wop_v, wot_v, t32,
            k_ref, qt_ref, vt_ref, s_a, s_b, ot_ref, h_ref, out_v, z_ref,
            in_sems, out_sems):
    nxb = S // TB
    cp_x0 = pltpu.make_async_copy(x_hbm.at[:, pl.ds(0, TB)], x_v.at[:, pl.ds(0, TB)], in_sems.at[0])
    cp_x1 = pltpu.make_async_copy(x_hbm.at[:, pl.ds(TB, S - TB)], x_v.at[:, pl.ds(TB, S - TB)], in_sems.at[1])
    cp_wqkv = pltpu.make_async_copy(wqkv_hbm, wqkv_v, in_sems.at[2])
    cp_wo = pltpu.make_async_copy(wo_hbm, wo_v, in_sems.at[3])
    cp_w1 = pltpu.make_async_copy(w1_hbm, w1_v, in_sems.at[4])
    cp_w3 = pltpu.make_async_copy(w3_hbm, w3_v, in_sems.at[5])
    cp_w2 = pltpu.make_async_copy(w2_hbm, w2_v, in_sems.at[6])
    cp_x0.start()
    cp_wqkv.start()
    z_ref[0] = 0
    z_ref[1] = 0

    def layernorm(b):
        cols = slice(b * TB, (b + 1) * TB)
        x = x_v[:, cols].astype(f32)
        mu = jnp.mean(x, axis=0, keepdims=True)
        xc = x - mu
        var = jnp.mean(xc * xc, axis=0, keepdims=True)
        xnt = (xc * jax.lax.rsqrt(var + EPS)).astype(bf16)
        xn = xnt.T
        xn_v[cols, :] = xn
        return xnt, xn

    z4w = jnp.zeros((HP - DH, D), f32)

    def pad_heads(dst, src32):
        for h in range(H):
            dst[HP * h:HP * (h + 1), :] = jnp.concatenate(
                [src32[DH * h:DH * (h + 1), :], z4w], axis=0).astype(bf16)

    row4 = jax.lax.broadcasted_iota(jnp.int32, (HP - DH, TB), 0)
    z4 = jnp.zeros((HP - DH, TB), f32)
    one4 = jnp.where(row4 == 0, 1.0, 0.0).astype(f32)

    def qv_proj(b, xnt):
        rows = slice(b * TB, (b + 1) * TB)
        qv = jnp.dot(wqv_v[...], xnt, preferred_element_type=f32)
        for h in range(H):
            q = qv[DH * h:DH * (h + 1)] * QSCALE
            qt_ref[h, :, rows] = jnp.concatenate([q, z4], axis=0).astype(bf16)
        for h in range(H):
            v = qv[D + DH * h:D + DH * (h + 1)]
            vt_ref[h, :, rows] = jnp.concatenate([v, one4], axis=0).astype(bf16)

    def k_proj(b, xn):
        rows = slice(b * TB, (b + 1) * TB)
        k = jax.lax.dot_general(xn, wk_v[...], _NT, preferred_element_type=f32)
        for g in range(G):
            k_ref[g, rows, :] = k[:, 128 * g:128 * (g + 1)].astype(bf16)

    cp_x0.wait()
    cp_x1.start()
    xnt, xn = layernorm(0)
    cp_wqkv.wait()
    cp_wo.start()
    cp_w1.start()
    cp_w3.start()
    cp_w2.start()
    wt = wqkv_v[...].T
    wqv_v[0:D, :] = wt[0:D]
    wqv_v[D:2 * D, :] = wt[2 * D:3 * D]
    t32[...] = wt[D:2 * D].astype(f32)
    pad_heads(wk_v, t32)
    qv_proj(0, xnt)
    cp_x1.wait()
    cp_wo.wait()
    k_proj(0, xn)
    for b in range(1, nxb):
        xnt, xn = layernorm(b)
        qv_proj(b, xnt)
        k_proj(b, xn)
    t32[...] = wo_v[...].astype(f32)
    pad_heads(wop_v, t32)
    wot_v[...] = wop_v[...].T
    cp_w1.wait()
    cp_w3.wait()
    cp_w2.wait()

    def out_copy(b):
        r0 = pl.multiple_of(b * BQ, BQ)
        return pltpu.make_async_copy(out_v.at[:, pl.ds(r0, BQ)],
                                     out_hbm.at[:, pl.ds(r0, BQ)], out_sems.at[b])

    NT = BQ // QT
    NITEM = NT * G

    def body(b, carry):
        q0 = pl.multiple_of(b * BQ, BQ)
        zs = pl.multiple_of(z_ref[0], 8)
        zl = pl.multiple_of(z_ref[1], 8)

        def q_weights(it):
            t, g = it // G, it % G
            cols = []
            for j in range(4):
                qj = qt_ref[4 * g + j, :, pl.ds(q0 + t * QT, QT)]
                parts = []
                if j > 0:
                    parts.append(jnp.zeros((HP * j, QT), bf16))
                parts.append(qj)
                if j < 3:
                    parts.append(jnp.zeros((HP * (3 - j), QT), bf16))
                cols.append(jnp.concatenate(parts, axis=0))
            return jnp.concatenate(cols, axis=1)

        def qk_chunk(it, c, qm, mrun):
            g = it % G
            sbuf = s_a if it % 2 == 0 else s_b
            s = jnp.dot(k_ref[g, c * C:(c + 1) * C, :], qm, preferred_element_type=f32)
            sbuf[pl.ds(zs + c * C, C), :] = s
            mc = jnp.max(s.reshape(C // 8, 8, W), axis=0)
            return mc if mrun is None else jnp.maximum(mrun, mc)

        def pv_chunk(it, c, m, o):
            g = it % G
            sbuf = s_a if it % 2 == 0 else s_b
            oc = []
            for j in range(4):
                cs = slice(j * QT, (j + 1) * QT)
                p = jnp.exp2(sbuf[pl.ds(zl + c * C, C), cs] - m[:, cs]).astype(bf16)
                oc.append(jnp.dot(vt_ref[4 * g + j, :, c * C:(c + 1) * C], p,
                                  preferred_element_type=f32))
            return oc if o is None else [a + b_ for a, b_ in zip(o, oc)]

        def ffn_chunk(c):
            xn = xn_v[pl.ds(q0, BQ), :]
            cols = slice(c * FC, (c + 1) * FC)
            gate = jnp.dot(xn, w1_v[:, cols], preferred_element_type=f32)
            up = jnp.dot(xn, w3_v[:, cols], preferred_element_type=f32)
            hg = 0.5 * gate
            h_ref[:, cols] = ((hg * jnp.tanh(hg) + hg) * up).astype(bf16)

        mrun = None
        qm = q_weights(0)
        for c in range(NC):
            mrun = qk_chunk(0, c, qm, mrun)
        m = jnp.max(mrun, axis=0, keepdims=True)
        nffn = F // FC
        for it in range(NITEM):
            mrun = None
            o = None
            if it + 1 < NITEM:
                qm = q_weights(it + 1)
                for c in range(NC + LAG):
                    if c < NC:
                        mrun = qk_chunk(it + 1, c, qm, mrun)
                    if c >= LAG:
                        o = pv_chunk(it, c - LAG, m, o)
                m = jnp.max(mrun, axis=0, keepdims=True)
            else:
                per = NC // NTAIL
                for c in range(NC):
                    if c % per == 0:
                        ffn_chunk(c // per)
                    o = pv_chunk(it, c, m, o)
            t, g = it // G, it % G
            for j in range(4):
                inv = 1.0 / o[j][DH:DH + 1, :]
                ot_ref[4 * g + j, :, t * QT:(t + 1) * QT] = (o[j] * inv).astype(bf16)
        for c in range(NTAIL, nffn):
            ffn_chunk(c)
        ot = ot_ref[...].reshape(H * HP, BQ)
        acc = jnp.dot(wot_v[...], ot, preferred_element_type=f32)
        acc = acc + jax.lax.dot_general(w2_v[...], h_ref[...], _NT,
                                        preferred_element_type=f32)
        acc = acc + x_v[:, pl.ds(q0, BQ)].astype(f32)
        out_v[:, pl.ds(q0, BQ)] = acc.astype(bf16)
        out_copy(b).start()
        return carry

    jax.lax.fori_loop(0, S // BQ, body, 0)
    for b in range(S // BQ):
        out_copy(b).wait()


@jax.jit
def pallas_parallel_sum__softmax_full_mha__glu_gated_swiglu__prompt_kernel(
    A_x, A_wqkv, A_wo, B_x, B_w1, B_w3, B_w2,
):
    del B_x
    xt = A_x.reshape(S, D).T
    any_spec = pl.BlockSpec(memory_space=pltpu.MemorySpace.HBM)
    out = pl.pallas_call(
        _kernel,
        out_shape=jax.ShapeDtypeStruct((D, S), bf16),
        in_specs=[any_spec] * 6,
        out_specs=any_spec,
        scratch_shapes=[
            pltpu.VMEM((D, S), bf16),
            pltpu.VMEM((D, 3 * D), bf16),
            pltpu.VMEM((D, D), bf16),
            pltpu.VMEM((D, F), bf16),
            pltpu.VMEM((D, F), bf16),
            pltpu.VMEM((D, F), bf16),
            pltpu.VMEM((S, D), bf16),
            pltpu.VMEM((2 * D, D), bf16),
            pltpu.VMEM((H * HP, D), bf16),
            pltpu.VMEM((H * HP, D), bf16),
            pltpu.VMEM((D, H * HP), bf16),
            pltpu.VMEM((D, D), f32),
            pltpu.VMEM((G, S, 128), bf16),
            pltpu.VMEM((H, HP, S), bf16),
            pltpu.VMEM((H, HP, S), bf16),
            pltpu.VMEM((S, W), f32),
            pltpu.VMEM((S, W), f32),
            pltpu.VMEM((H, HP, BQ), bf16),
            pltpu.VMEM((BQ, F), bf16),
            pltpu.VMEM((D, S), bf16),
            pltpu.SMEM((2,), jnp.int32),
            pltpu.SemaphoreType.DMA((7,)),
            pltpu.SemaphoreType.DMA((S // BQ,)),
        ],
        compiler_params=pltpu.CompilerParams(vmem_limit_bytes=100 * 1024 * 1024),
    )(xt, A_wqkv, A_wo, B_w1, B_w3, B_w2.T)
    return out.T.reshape(1, S, D)
```

```python
import math

import jax
import jax.numpy as jnp
import jax.experimental.pallas as pl
import jax.experimental.pallas.tpu as pltpu

S = 2048
D = 448
H = 16
DH = D // H
F = 1792
G = 4
HP = 32
QT = 128
W = 4 * QT
BQ = 256
NT = BQ // QT
NITEM = NT * G
C = 128
NC = S // C
LAG = 2
TT = 128
FC = 128
NFFN = F // FC
NTAIL = 2
NHEAD = NFFN - NTAIL
NOFF = 96
X0 = 512
WA = 512
EPS = 1e-5
QSCALE = (DH ** -0.5) * math.log2(math.e)

_NT_DIMS = (((1,), (1,)), ((), ()))
f32 = jnp.float32
bf16 = jnp.bfloat16
u32 = jnp.uint32


def _pk(x):
    return pltpu.bitcast(x, u32)


def _up(x):
    return pltpu.bitcast(x, bf16)


def _kernel(x_hbm, wqkv_hbm, wo_hbm, w1_hbm, w3_hbm, w2_hbm, out_hbm,
            x_v, wqkv_v, wo_v, w1_v, w3_v, w2_v,
            xn_p, xc_p, wt_p, wot_p, kt32,
            k_p, qt_p, q32_ref, vt_p, kb_ref, s_a, s_b, sv0, sv1, sv2, sv3,
            ot_p, h_p, acc_ref, out_v, z_ref, in_sems, out_sems):
    svs = [sv0, sv1, sv2, sv3]

    def cols_copy(src, dst, lo, n, sem):
        return pltpu.make_async_copy(src.at[:, pl.ds(lo, n)], dst.at[:, pl.ds(lo, n)], sem)

    cp_x0 = cols_copy(x_hbm, x_v, 0, X0, in_sems.at[0])
    cp_x1 = cols_copy(x_hbm, x_v, X0, S - X0, in_sems.at[1])
    cp_wa = cols_copy(wqkv_hbm, wqkv_v, 0, WA, in_sems.at[2])
    cp_wb = cols_copy(wqkv_hbm, wqkv_v, WA, 3 * D - WA, in_sems.at[3])
    cp_wo = pltpu.make_async_copy(wo_hbm, wo_v, in_sems.at[4])
    cp_w1 = pltpu.make_async_copy(w1_hbm, w1_v, in_sems.at[5])
    cp_w3 = pltpu.make_async_copy(w3_hbm, w3_v, in_sems.at[6])
    cp_w2 = pltpu.make_async_copy(w2_hbm, w2_v, in_sems.at[7])
    cp_x0.start()
    cp_wa.start()
    cp_wb.start()
    cp_x1.start()
    z_ref[0] = 0
    z_ref[1] = 0

    def layernorm(n):
        x = x_v[:, n * TT:(n + 1) * TT].astype(f32)
        mu = jnp.mean(x, axis=0, keepdims=True)
        xc = x - mu
        var = jnp.mean(xc * xc, axis=0, keepdims=True)
        xnt = (xc * jax.lax.rsqrt(var + EPS)).astype(bf16)
        xn_p[n * TT // 2:(n + 1) * TT // 2, :] = _pk(xnt.T)
        return xnt

    row4 = jax.lax.broadcasted_iota(jnp.int32, (HP - DH, TT), 0)
    z4 = jnp.zeros((HP - DH, TT), f32)
    one4 = jnp.where(row4 == 0, 1.0, 0.0).astype(f32)

    def qkv_proj(n, xnt, do_q=True, do_kv=True):
        cols = slice(n * TT, (n + 1) * TT)
        r0 = 0 if do_q else D
        r1 = 3 * D if do_kv else D
        qkv = jnp.dot(_up(wt_p[r0 // 2:r1 // 2, :]), xnt, preferred_element_type=f32)
        if do_q:
            for h in range(H):
                q = qkv[DH * h:DH * (h + 1)] * QSCALE
                qt_p[h, :, cols] = _pk(jnp.concatenate([q, z4], axis=0).astype(bf16))
        if do_kv:
            ko = D - r0
            vo = 2 * D - r0
            for g in range(G):
                parts = []
                for j in range(4):
                    h = 4 * g + j
                    parts += [qkv[ko + DH * h:ko + DH * (h + 1)], z4]
                k_p[g, n * TT // 2:(n + 1) * TT // 2, :] = _pk(
                    jnp.concatenate(parts, axis=0).astype(bf16).T)
            if n == 0:
                kt32[...] = qkv[ko:ko + D]
            for h in range(H):
                v = qkv[vo + DH * h:vo + DH * (h + 1)]
                vt_p[h, :, cols] = _pk(jnp.concatenate([v, one4], axis=0).astype(bf16))

    def kb_gen(lo, hi):
        for r in range(lo, hi):
            kb = jnp.broadcast_to(kt32[r:r + 1, :], (TT, TT)).astype(bf16).T
            kb_ref[r] = kb[0:NOFF].astype(f32)

    ntile = S // TT
    n0 = X0 // TT
    cp_x0.wait()
    xnts = [layernorm(n) for n in range(n0)]
    cp_wa.wait()
    wt_p[0:WA // 2, :] = _pk(wqkv_v[:, 0:WA].T)
    for n in range(n0 - 1):
        qkv_proj(n, xnts[n], do_kv=False)
    cp_wb.wait()
    cp_wo.start()
    cp_w1.start()
    cp_w3.start()
    cp_w2.start()
    wt_p[WA // 2:3 * D // 2, :] = _pk(wqkv_v[:, WA:3 * D].T)
    qkv_proj(n0 - 1, xnts[n0 - 1], do_kv=False)
    nkb = ntile - 2
    for n in range(ntile):
        if n == n0 - 1:
            cp_x1.wait()
            cp_wo.wait()
        xnt = xnts[n] if n < n0 else layernorm(n)
        qkv_proj(n, xnt, do_q=(n >= n0))
        if 1 <= n < 1 + nkb:
            kb_gen((n - 1) * D // nkb, n * D // nkb)
        if n == ntile - 2:
            wo32 = wo_v[...].astype(f32)
            z4w = jnp.zeros((HP - DH, D), f32)
            parts = []
            for h in range(H):
                parts += [wo32[DH * h:DH * (h + 1), :], z4w]
            wot_p[...] = _pk(jnp.concatenate(parts, axis=0).astype(bf16).T)
    cp_w1.wait()
    cp_w3.wait()
    cp_w2.wait()

    def out_copy(b):
        r0 = pl.multiple_of(b * BQ, BQ)
        return pltpu.make_async_copy(out_v.at[:, pl.ds(r0, BQ)],
                                     out_hbm.at[:, pl.ds(r0, BQ)], out_sems.at[b])

    qk_ranges = [(max(c * C, NOFF), (c + 1) * C) for c in range(NC)]

    def body(b, carry):
        q0 = pl.multiple_of(b * BQ, BQ)
        zs = pl.multiple_of(z_ref[0], 8)
        zl = pl.multiple_of(z_ref[1], 8)
        never = jax.lax.broadcasted_iota(jnp.int32, (8, QT), 1) < z_ref[0]

        for h in reversed(range(H)):
            q32_ref[h] = _up(qt_p[h, :, pl.ds(q0, BQ)]).astype(f32)
        xc_p[...] = xn_p[pl.ds(pl.multiple_of(b * (BQ // 2), BQ // 2), BQ // 2), :]

        def q_weights(it):
            g, t = it // NT, it % NT
            cols = []
            for j in range(4):
                qj = _up(qt_p[4 * g + j, :, pl.ds(q0 + t * QT, QT)])
                parts = []
                if j > 0:
                    parts.append(jnp.zeros((HP * j, QT), bf16))
                parts.append(qj)
                if j < 3:
                    parts.append(jnp.zeros((HP * (3 - j), QT), bf16))
                cols.append(jnp.concatenate(parts, axis=0))
            return jnp.concatenate(cols, axis=1)

        def qk_chunk(it, c, qm, mrun):
            g = it // NT
            lo, hi = qk_ranges[c]
            sbuf = s_a if it % 2 == 0 else s_b
            s = jnp.dot(_up(k_p[g, lo // 2:hi // 2, :]), qm, preferred_element_type=f32)
            sbuf[pl.ds(zs + lo, hi - lo), :] = s
            mc = jnp.max(s.reshape((hi - lo) // 8, 8, W), axis=0)
            return mc if mrun is None else jnp.maximum(mrun, mc)

        def vpu_scores():
            chain = [None] * NT
            for h in reversed(range(H)):
                g, j = h // 4, h % 4
                cs = slice(j * QT, (j + 1) * QT)
                vmax = [None] * NT
                for r in range(NOFF // 8):
                    acc = [None] * NT
                    for d in range(DH):
                        kb = kb_ref[DH * h + d, r * 8:(r + 1) * 8, :]
                        for t in range(NT):
                            prod = kb * q32_ref[h, d:d + 1, t * QT:(t + 1) * QT]
                            if acc[t] is not None:
                                acc[t] = acc[t] + prod
                            elif chain[t] is None:
                                acc[t] = prod
                            else:
                                acc[t] = jnp.where(never, chain[t], prod)
                    for t in range(NT):
                        chain[t] = acc[t]
                        svs[g][t, pl.ds(zs + r * 8, 8), cs] = acc[t]
                        vmax[t] = acc[t] if vmax[t] is None else jnp.maximum(vmax[t], acc[t])
                for t in range(NT):
                    svs[g][t, pl.ds(zs + NOFF, 8), cs] = vmax[t]

        def final_max(it, mrun):
            mrun = jnp.maximum(mrun, svs[it // NT][it % NT, pl.ds(zl + NOFF, 8), :])
            return jnp.max(mrun, axis=0, keepdims=True)

        def pv_chunk(it, c, m, o):
            g = it // NT
            sbuf = s_a if it % 2 == 0 else s_b
            lo, hi = qk_ranges[c]
            oc = []
            for j in range(4):
                cs = slice(j * QT, (j + 1) * QT)
                s = sbuf[pl.ds(zl + lo, hi - lo), cs]
                if c == 0:
                    s = jnp.concatenate([svs[g][it % NT, pl.ds(zl, NOFF), cs], s], axis=0)
                p = jnp.exp2(s - m[:, cs]).astype(bf16)
                oc.append(jnp.dot(_up(vt_p[4 * g + j, :, c * C:(c + 1) * C]), p,
                                  preferred_element_type=f32))
            return oc if o is None else [a + e for a, e in zip(o, oc)]

        def ffn_gate(c, r0=0, n=BQ):
            xn = _up(xc_p[r0 // 2:(r0 + n) // 2, :])
            gate = jnp.dot(xn, w1_v[:, c * FC:(c + 1) * FC], preferred_element_type=f32)
            hg = 0.5 * gate
            return hg * jnp.tanh(hg) + hg

        def ffn_up(c, act, r0=0, n=BQ):
            xn = _up(xc_p[r0 // 2:(r0 + n) // 2, :])
            cols = slice(c * FC, (c + 1) * FC)
            up = jnp.dot(xn, w3_v[:, cols], preferred_element_type=f32)
            h_p[r0 // 2:(r0 + n) // 2, cols] = _pk((act * up).astype(bf16))

        def ffn_down(lo, hi):
            return jax.lax.dot_general(w2_v[:, lo:hi], _up(h_p[:, lo:hi]), _NT_DIMS,
                                       preferred_element_type=f32)

        def wo_proj(lo, hi, r0=0, n=D):
            ot = _up(ot_p[lo:hi].reshape((hi - lo) * HP // 2, BQ))
            return jnp.dot(_up(wot_p[r0 // 2:(r0 + n) // 2, lo * HP:hi * HP]), ot,
                           preferred_element_type=f32)

        vpu_scores()
        for c in range(NHEAD):
            ffn_up(c, ffn_gate(c))
        mrun = None
        qm = q_weights(0)
        for c in range(NC):
            mrun = qk_chunk(0, c, qm, mrun)
        acc_ref[pl.ds(zs, D), :] = (ffn_down(0, NHEAD * FC)
                                    + x_v[:, pl.ds(q0, BQ)].astype(f32))
        m = final_max(0, mrun)
        acc = None
        for it in range(NITEM):
            mrun = None
            o = None
            if it + 1 < NITEM:
                qm = q_weights(it + 1)
                for ci in range(NC + LAG):
                    if ci < NC:
                        mrun = qk_chunk(it + 1, ci, qm, mrun)
                    if ci >= LAG:
                        o = pv_chunk(it, ci - LAG, m, o)
                m = final_max(it + 1, mrun)
            else:
                fill = []
                for c in range(NHEAD, NFFN):
                    for i in range(NT):
                        fill.append(("gate", c, i))
                        fill.append(("up", c, i))
                nws = 4
                fill += [("wo", 0, i) for i in range(nws)]
                accs = []
                act = None
                for c in range(NC):
                    for k, (kind, fc, i) in enumerate(fill):
                        if k * NC // len(fill) != c:
                            continue
                        if kind == "gate":
                            act = ffn_gate(fc, i * QT, QT)
                        elif kind == "up":
                            ffn_up(fc, act, i * QT, QT)
                        else:
                            r0, n = i * D // nws, D // nws
                            accs.append(acc_ref[pl.ds(zl + r0, n), :] + wo_proj(0, H // 2, r0, n))
                    o = pv_chunk(it, c, m, o)
                acc = jnp.concatenate(accs, axis=0) + ffn_down(NHEAD * FC, F)
            g, t = it // NT, it % NT
            for j in range(4):
                inv = 1.0 / o[j][DH:DH + 1, :]
                ot_p[4 * g + j, :, t * QT:(t + 1) * QT] = _pk((o[j] * inv).astype(bf16))
        acc = acc + wo_proj(H // 2, H)
        out_v[:, pl.ds(q0, BQ)] = acc.astype(bf16)
        out_copy(b).start()
        return carry

    jax.lax.fori_loop(0, S // BQ, body, 0)
    for b in range(S // BQ):
        out_copy(b).wait()


@jax.jit
def pallas_parallel_sum__softmax_full_mha__glu_gated_swiglu__prompt_kernel(
    A_x: jax.Array,
    A_wqkv: jax.Array,
    A_wo: jax.Array,
    B_x: jax.Array,
    B_w1: jax.Array,
    B_w3: jax.Array,
    B_w2: jax.Array,
):
    del B_x
    xt = A_x.reshape(S, D).T
    hbm_spec = pl.BlockSpec(memory_space=pltpu.MemorySpace.HBM)
    sv_shape = pltpu.VMEM((NT, NOFF + 8, W), f32)
    out = pl.pallas_call(
        _kernel,
        out_shape=jax.ShapeDtypeStruct((D, S), bf16),
        in_specs=[hbm_spec] * 6,
        out_specs=hbm_spec,
        scratch_shapes=[
            pltpu.VMEM((D, S), bf16),
            pltpu.VMEM((D, 3 * D), bf16),
            pltpu.VMEM((D, D), bf16),
            pltpu.VMEM((D, F), bf16),
            pltpu.VMEM((D, F), bf16),
            pltpu.VMEM((D, F), bf16),
            pltpu.VMEM((S // 2, D), u32),
            pltpu.VMEM((BQ // 2, D), u32),
            pltpu.VMEM((3 * D // 2, D), u32),
            pltpu.VMEM((D // 2, H * HP), u32),
            pltpu.VMEM((D, TT), f32),
            pltpu.VMEM((G, S // 2, 128), u32),
            pltpu.VMEM((H, HP // 2, S), u32),
            pltpu.VMEM((H, HP, BQ), f32),
            pltpu.VMEM((H, HP // 2, S), u32),
            pltpu.VMEM((D, NOFF, 128), f32),
            pltpu.VMEM((S, W), f32),
            pltpu.VMEM((S, W), f32),
            sv_shape, sv_shape, sv_shape, sv_shape,
            pltpu.VMEM((H, HP // 2, BQ), u32),
            pltpu.VMEM((BQ // 2, F), u32),
            pltpu.VMEM((D, BQ), f32),
            pltpu.VMEM((D, S), bf16),
            pltpu.SMEM((2,), jnp.int32),
            pltpu.SemaphoreType.DMA((8,)),
            pltpu.SemaphoreType.DMA((S // BQ,)),
        ],
        compiler_params=pltpu.CompilerParams(vmem_limit_bytes=100 * 1024 * 1024),
    )(xt, A_wqkv, A_wo, B_w1, B_w3, B_w2.T)
    return out.T.reshape(1, S, D)
```

```python
import math

import jax
import jax.numpy as jnp
import jax.experimental.pallas as pl
import jax.experimental.pallas.tpu as pltpu

S = 2048
D = 448
H = 16
DH = D // H
F = 1792
G = 4
HP = 32
QT = 128
W = 4 * QT
BQ = 256
NT = BQ // QT
NITEM = NT * G
C = 128
NC = S // C
LAG = 3
TT = 128
FC = 128
NFFN = F // FC
NTAIL = 2
NHEAD = NFFN - NTAIL
QK0_SPREAD = (2, 2, 2, 2, 2, 2, 3)
X0 = 512
WA = 512
QR = H * HP
SVR = C + 8
EPS = 1e-5
QSCALE = (DH ** -0.5) * math.log2(math.e)

_NT_DIMS = (((1,), (1,)), ((), ()))
f32 = jnp.float32
bf16 = jnp.bfloat16
u32 = jnp.uint32


def _pk(x):
    return pltpu.bitcast(x, u32)


def _up(x):
    return pltpu.bitcast(x, bf16)


def _kernel(x_hbm, wqkv_hbm, wo_hbm, w1_hbm, w3_hbm, w2_hbm, out_hbm,
            x_v, wqkv_v, wo_v, w1_v, w3_v, w2_v,
            xn_p, xc_p, wt_p, wot_p, kt32,
            k_p, qt_p, qs_ref, vt_p, kb_ref, s_a, s_b,
            ot_p, h_p, acc_ref, out_v, z_ref, sems):
    def cols_copy(src, dst, lo, n, sem):
        return pltpu.make_async_copy(src.at[:, pl.ds(lo, n)], dst.at[:, pl.ds(lo, n)], sem)

    cp_x0 = cols_copy(x_hbm, x_v, 0, X0, sems.at[0])
    cp_wa = cols_copy(wqkv_hbm, wqkv_v, 0, WA, sems.at[1])
    cp_wb = cols_copy(wqkv_hbm, wqkv_v, WA, 3 * D - WA, sems.at[2])
    cp_x1 = cols_copy(x_hbm, x_v, X0, S - X0, sems.at[3])
    cp_wo = pltpu.make_async_copy(wo_hbm, wo_v, sems.at[3])
    cp_w1 = pltpu.make_async_copy(w1_hbm, w1_v, sems.at[4])
    cp_w3 = pltpu.make_async_copy(w3_hbm, w3_v, sems.at[4])
    cp_w2 = pltpu.make_async_copy(w2_hbm, w2_v, sems.at[4])
    cp_x0.start()
    cp_wa.start()
    cp_wb.start()
    cp_x1.start()
    z_ref[0] = 0
    z_ref[1] = 0

    false_row = []

    def layernorm(n, pin=None):
        x = x_v[:, n * TT:(n + 1) * TT].astype(f32)
        if pin is not None:
            x = jnp.concatenate([jnp.where(false_row[0], pin, x[0:8]), x[8:]], axis=0)
        mu = jnp.mean(x, axis=0, keepdims=True)
        xc = x - mu
        var = jnp.mean(xc * xc, axis=0, keepdims=True)
        if not false_row:
            false_row.append(var < -1.0)
        xnt = (xc * jax.lax.rsqrt(var + EPS)).astype(bf16)
        xn_p[n * TT // 2:(n + 1) * TT // 2, :] = _pk(xnt.T)
        return xnt

    row4 = jax.lax.broadcasted_iota(jnp.int32, (HP - DH, TT), 0)
    z4 = jnp.zeros((HP - DH, TT), f32)
    one4 = jnp.where(row4 == 0, 1.0, 0.0).astype(f32)

    def qkv_proj(n, xnt, do_q=True, do_kv=True):
        cols = slice(n * TT, (n + 1) * TT)
        r0 = 0 if do_q else D
        r1 = 3 * D if do_kv else D
        qkv = jnp.dot(_up(wt_p[r0 // 2:r1 // 2, :]), xnt, preferred_element_type=f32)
        if do_q:
            for h in range(H):
                q = qkv[DH * h:DH * (h + 1)] * QSCALE
                qt_p[h, :, cols] = _pk(jnp.concatenate([q, z4], axis=0).astype(bf16))
        if do_kv:
            ko = D - r0
            vo = 2 * D - r0
            for g in range(G):
                parts = []
                for j in range(4):
                    h = 4 * g + j
                    parts += [qkv[ko + DH * h:ko + DH * (h + 1)], z4]
                k_p[g, n * TT // 2:(n + 1) * TT // 2, :] = _pk(
                    jnp.concatenate(parts, axis=0).astype(bf16).T)
            if n == 0:
                kt32[...] = qkv[ko:ko + D]
            for h in range(H):
                v = qkv[vo + DH * h:vo + DH * (h + 1)]
                vt_p[h, :, cols] = _pk(jnp.concatenate([v, one4], axis=0).astype(bf16))
        late = (r1 - r0) * 5 // 64 * 8
        return qkv[0:8], qkv[late:late + 8]

    def kb_gen(lo, hi, pin):
        for r in range(lo, hi):
            row8 = jnp.where(false_row[0], pin, jnp.broadcast_to(kt32[r:r + 1, :], (8, TT)))
            kb = jnp.concatenate([row8] * (TT // 8), axis=0).astype(bf16).T
            kb_ref[r] = kb.astype(f32)

    ntile = S // TT
    n0 = X0 // TT
    cp_x0.wait()
    xnts = [layernorm(n) for n in range(n0)]
    cp_wa.wait()
    wt_p[0:WA // 2, :] = _pk(wqkv_v[:, 0:WA].T)
    for n in range(n0 - 1):
        qkv_proj(n, xnts[n], do_kv=False)
    cp_wb.wait()
    cp_wo.start()
    cp_w1.start()
    cp_w3.start()
    cp_w2.start()
    wt_p[WA // 2:3 * D // 2, :] = _pk(wqkv_v[:, WA:3 * D].T)
    qkv_proj(n0 - 1, xnts[n0 - 1], do_kv=False)
    nkb = ntile - 2
    pins = []
    for n in range(ntile):
        if n == n0 - 1:
            cp_x1.wait()
            cp_wo.wait()
        xnt = xnts[n] if n < n0 else layernorm(n, pins[n - 2][1])
        pins.append(qkv_proj(n, xnt, do_q=(n >= n0)))
        if 1 <= n < 1 + nkb:
            kb_gen((n - 1) * D // nkb, n * D // nkb, pins[n][0])
        if n == ntile - 2:
            wo32 = wo_v[...].astype(f32)
            z4w = jnp.zeros((HP - DH, D), f32)
            parts = []
            for h in range(H):
                parts += [wo32[DH * h:DH * (h + 1), :], z4w]
            wot_p[...] = _pk(jnp.concatenate(parts, axis=0).astype(bf16).T)
    cp_w1.wait()
    cp_w3.wait()
    cp_w2.wait()

    def out_copy(b):
        r0 = pl.multiple_of(b * BQ, BQ)
        return pltpu.make_async_copy(out_v.at[:, pl.ds(r0, BQ)],
                                     out_hbm.at[:, pl.ds(r0, BQ)], sems.at[5])

    def body(b, carry):
        q0 = pl.multiple_of(b * BQ, BQ)
        zs = pl.multiple_of(z_ref[0], 8)
        zl = pl.multiple_of(z_ref[1], 8)
        never = jax.lax.broadcasted_iota(jnp.int32, (2, 8, QT), 2) < z_ref[0]

        for h in reversed(range(H)):
            qs_ref[HP * h:HP * (h + 1), :] = _up(qt_p[h, :, pl.ds(q0, BQ)]).astype(f32)
        xc_p[...] = xn_p[pl.ds(pl.multiple_of(b * (BQ // 2), BQ // 2), BQ // 2), :]

        def q_weights(it):
            g, t = it // NT, it % NT
            cols = []
            for j in range(4):
                qj = _up(qt_p[4 * g + j, :, pl.ds(q0 + t * QT, QT)])
                parts = []
                if j > 0:
                    parts.append(jnp.zeros((HP * j, QT), bf16))
                parts.append(qj)
                if j < 3:
                    parts.append(jnp.zeros((HP * (3 - j), QT), bf16))
                cols.append(jnp.concatenate(parts, axis=0))
            return jnp.concatenate(cols, axis=1)

        def qk_chunk(it, c, qm, mrun):
            sbuf = s_a if it % 2 == 0 else s_b
            s = jnp.dot(_up(k_p[it // NT, c * C // 2:(c + 1) * C // 2, :]), qm,
                        preferred_element_type=f32)
            sbuf[pl.ds(zs + c * C, C), :] = s
            mc = jnp.max(s.reshape(C // 8, 8, W), axis=0)
            return mc if mrun is None else jnp.maximum(mrun, mc)

        def vpu_scores():
            chain = None
            pending = []
            for t in reversed(range(NT)):
                cs = slice(t * QT, (t + 1) * QT)
                for h in reversed(range(H)):
                    qb = jnp.stack([jnp.broadcast_to(qs_ref[HP * h + d:HP * h + d + 1, cs], (8, QT))
                                    for d in range(DH)])[:, None]
                    vmax = None
                    for r in range(C // 16):
                        acc = None
                        for d in range(0, DH, 4):
                            kb = kb_ref[DH * h + d:DH * h + d + 4, r * 16:(r + 1) * 16, :]
                            prod = kb.reshape(4, 2, 8, QT) * qb[d:d + 4]
                            pair = prod[2:3] + prod[3:4]
                            if acc is not None:
                                terms = [acc[None], prod[0:2], pair]
                            elif chain is None:
                                terms = [prod[0:2], pair]
                            else:
                                terms = [jnp.where(never, chain, prod[0])[None], prod[1:2], pair]
                            acc = jnp.sum(jnp.concatenate(terms, axis=0), axis=0)
                        chain = acc
                        vmax = acc if vmax is None else jnp.maximum(vmax, acc)
                        pending.append((QR + h * SVR + r * 16, cs, acc.reshape(16, QT)))
                    pending.append((QR + h * SVR + C, cs, jnp.maximum(vmax[0], vmax[1])))
                    while len(pending) > 2:
                        row, cols, val = pending.pop(0)
                        qs_ref[pl.ds(zs + row, val.shape[0]), cols] = val
            for row, cols, val in pending:
                qs_ref[pl.ds(zs + row, val.shape[0]), cols] = val

        def final_max(it, mrun):
            g, t = it // NT, it % NT
            vm = jnp.concatenate(
                [qs_ref[QR + (4 * g + j) * SVR + C:QR + (4 * g + j + 1) * SVR, t * QT:(t + 1) * QT]
                 for j in range(4)], axis=1)
            return jnp.max(jnp.maximum(mrun, vm), axis=0, keepdims=True)

        def pv_chunk(it, c, m, o):
            g, t = it // NT, it % NT
            sbuf = s_a if it % 2 == 0 else s_b
            oc = []
            for j in range(4):
                cs = slice(j * QT, (j + 1) * QT)
                if c == 0:
                    r0 = QR + (4 * g + j) * SVR
                    s = qs_ref[r0:r0 + C, t * QT:(t + 1) * QT]
                else:
                    s = sbuf[pl.ds(zl + c * C, C), cs]
                p = jnp.exp2(s - m[:, cs]).astype(bf16)
                oc.append(jnp.dot(_up(vt_p[4 * g + j, :, c * C:(c + 1) * C]), p,
                                  preferred_element_type=f32))
            return oc if o is None else [a + e for a, e in zip(o, oc)]

        def ffn_gate(c, r0=0, n=BQ):
            xn = _up(xc_p[r0 // 2:(r0 + n) // 2, :])
            gate = jnp.dot(xn, w1_v[:, c * FC:(c + 1) * FC], preferred_element_type=f32)
            hg = 0.5 * gate
            return hg * jnp.tanh(hg) + hg

        def ffn_up(c, act, r0=0, n=BQ):
            xn = _up(xc_p[r0 // 2:(r0 + n) // 2, :])
            cols = slice(c * FC, (c + 1) * FC)
            up = jnp.dot(xn, w3_v[:, cols], preferred_element_type=f32)
            h_p[r0 // 2:(r0 + n) // 2, cols] = _pk((act * up).astype(bf16))

        def ffn_down(lo, hi):
            return jax.lax.dot_general(w2_v[:, lo:hi], _up(h_p[:, lo:hi]), _NT_DIMS,
                                       preferred_element_type=f32)

        def wo_proj(lo, hi, r0=0, n=D):
            ot = _up(ot_p[lo:hi].reshape((hi - lo) * HP // 2, BQ))
            return jnp.dot(_up(wot_p[r0 // 2:(r0 + n) // 2, lo * HP:hi * HP]), ot,
                           preferred_element_type=f32)

        vpu_scores()
        mrun = None
        qm = q_weights(0)
        dn = None
        nq = 1
        for i in range(NHEAD // 2 + 1):
            if i < NHEAD // 2:
                for c in (2 * i, 2 * i + 1):
                    ffn_up(c, ffn_gate(c))
            for c in range(nq, nq + QK0_SPREAD[i]):
                mrun = qk_chunk(0, c, qm, mrun)
            nq += QK0_SPREAD[i]
            if i > 0:
                part = ffn_down(2 * (i - 1) * FC, 2 * i * FC)
                dn = part if dn is None else dn + part
        assert nq == NC
        acc_ref[pl.ds(zs, D), :] = dn + x_v[:, pl.ds(q0, BQ)].astype(f32)
        m = final_max(0, mrun)

        acc = None
        for it in range(NITEM):
            mrun = None
            o = None
            if it + 1 < NITEM:
                qm = q_weights(it + 1)
                nslot = NC - LAG
                pv = 0
                for c in range(1, NC):
                    mrun = qk_chunk(it + 1, c, qm, mrun)
                    if c >= LAG:
                        while pv < ((c - LAG + 1) * (NC - 1)) // nslot:
                            o = pv_chunk(it, pv, m, o)
                            pv += 1
                o = pv_chunk(it, NC - 1, m, o)
                m = final_max(it + 1, mrun)
            else:
                fill = []
                for c in range(NHEAD, NFFN):
                    for i in range(NT):
                        fill.append(("gate", c, i))
                        fill.append(("up", c, i))
                nws = 4
                fill += [("wo", 0, i) for i in range(nws)]
                accs = []
                act = None
                for c in range(NC):
                    for k, (kind, fc, i) in enumerate(fill):
                        if k * NC // len(fill) != c:
                            continue
                        if kind == "gate":
                            act = ffn_gate(fc, i * QT, QT)
                        elif kind == "up":
                            ffn_up(fc, act, i * QT, QT)
                        else:
                            r0, n = i * D // nws, D // nws
                            accs.append(acc_ref[pl.ds(zl + r0, n), :] + wo_proj(0, H // 2, r0, n))
                    o = pv_chunk(it, c, m, o)
                acc = jnp.concatenate(accs, axis=0) + ffn_down(NHEAD * FC, F)
            g, t = it // NT, it % NT
            for j in range(4):
                inv = 1.0 / o[j][DH:DH + 1, :]
                ot_p[4 * g + j, :, t * QT:(t + 1) * QT] = _pk((o[j] * inv).astype(bf16))
        acc = acc + wo_proj(H // 2, H)
        out_v[:, pl.ds(q0, BQ)] = acc.astype(bf16)
        out_copy(b).start()
        return carry

    jax.lax.fori_loop(0, S // BQ, body, 0)
    for b in range(S // BQ):
        out_copy(b).wait()


@jax.jit
def pallas_parallel_sum__softmax_full_mha__glu_gated_swiglu__prompt_kernel(
    A_x: jax.Array,
    A_wqkv: jax.Array,
    A_wo: jax.Array,
    B_x: jax.Array,
    B_w1: jax.Array,
    B_w3: jax.Array,
    B_w2: jax.Array,
):
    del B_x
    xt = A_x.reshape(S, D).T
    hbm_spec = pl.BlockSpec(memory_space=pltpu.MemorySpace.HBM)
    out = pl.pallas_call(
        _kernel,
        out_shape=jax.ShapeDtypeStruct((D, S), bf16),
        in_specs=[hbm_spec] * 6,
        out_specs=hbm_spec,
        scratch_shapes=[
            pltpu.VMEM((D, S), bf16),
            pltpu.VMEM((D, 3 * D), bf16),
            pltpu.VMEM((D, D), bf16),
            pltpu.VMEM((D, F), bf16),
            pltpu.VMEM((D, F), bf16),
            pltpu.VMEM((D, F), bf16),
            pltpu.VMEM((S // 2, D), u32),
            pltpu.VMEM((BQ // 2, D), u32),
            pltpu.VMEM((3 * D // 2, D), u32),
            pltpu.VMEM((D // 2, H * HP), u32),
            pltpu.VMEM((D, TT), f32),
            pltpu.VMEM((G, S // 2, 128), u32),
            pltpu.VMEM((H, HP // 2, S), u32),
            pltpu.VMEM((QR + H * SVR, BQ), f32),
            pltpu.VMEM((H, HP // 2, S), u32),
            pltpu.VMEM((D, C, 128), f32),
            pltpu.VMEM((S, W), f32),
            pltpu.VMEM((S, W), f32),
            pltpu.VMEM((H, HP // 2, BQ), u32),
            pltpu.VMEM((BQ // 2, F), u32),
            pltpu.VMEM((D, BQ), f32),
            pltpu.VMEM((D, S), bf16),
            pltpu.SMEM((2,), jnp.int32),
            pltpu.SemaphoreType.DMA((6,)),
        ],
        compiler_params=pltpu.CompilerParams(vmem_limit_bytes=100 * 1024 * 1024),
    )(xt, A_wqkv, A_wo, B_w1, B_w3, B_w2.T)
    return out.T.reshape(1, S, D)
```

```python
import math

import jax
import jax.numpy as jnp
import jax.experimental.pallas as pl
import jax.experimental.pallas.tpu as pltpu

S = 2048
D = 448
H = 16
DH = D // H
F = 1792
G = 4
HP = 32
QT = 128
W = 4 * QT
BQ = 256
NT = BQ // QT
NITEM = NT * G
C = 128
NC = S // C
LAG = 3
TT = 128
FC = 128
NFFN = F // FC
NTAIL = 2
NHEAD = NFFN - NTAIL
QK0_SPREAD = (1, 2, 2, 2, 2, 3, 3)
Q_AHEAD = 3
NWS = 7
X0 = 512
WA = 512
QR = H * HP
SVR = C + 8
EPS = 1e-5
QSCALE = (DH ** -0.5) * math.log2(math.e)

_NT_DIMS = (((1,), (1,)), ((), ()))
f32 = jnp.float32
bf16 = jnp.bfloat16
u32 = jnp.uint32


def _pk(x):
    return pltpu.bitcast(x, u32)


def _up(x):
    return pltpu.bitcast(x, bf16)


def _kernel(x_hbm, wqkv_hbm, wo_hbm, w1_hbm, w3_hbm, w2_hbm, out_hbm,
            x_v, wqkv_v, wo_v, w1_v, w3_v, w2_v,
            xn_p, xc_p, wt_p, wot_p, kt32,
            k_p, qt_p, qs_ref, vt_p, kb_ref, s_a, s_b,
            ot_p, h_p, acc_ref, out_v, z_ref, sems):
    def cols_copy(src, dst, lo, n, sem):
        return pltpu.make_async_copy(src.at[:, pl.ds(lo, n)], dst.at[:, pl.ds(lo, n)], sem)

    cp_x0 = cols_copy(x_hbm, x_v, 0, X0, sems.at[0])
    cp_wa = cols_copy(wqkv_hbm, wqkv_v, 0, WA, sems.at[1])
    cp_wb = cols_copy(wqkv_hbm, wqkv_v, WA, 3 * D - WA, sems.at[2])
    cp_x1 = cols_copy(x_hbm, x_v, X0, S - X0, sems.at[3])
    cp_wo = pltpu.make_async_copy(wo_hbm, wo_v, sems.at[3])
    cp_w1 = pltpu.make_async_copy(w1_hbm, w1_v, sems.at[4])
    cp_w3 = pltpu.make_async_copy(w3_hbm, w3_v, sems.at[4])
    cp_w2 = pltpu.make_async_copy(w2_hbm, w2_v, sems.at[4])
    cp_x0.start()
    cp_wa.start()
    cp_wb.start()
    cp_x1.start()
    z_ref[0] = 0
    z_ref[1] = 0

    false_row = []

    def store_xn(n, xnt):
        xn_p[n * TT // 2:(n + 1) * TT // 2, :] = _pk(xnt.T)

    def layernorm(n, pin=None):
        x = x_v[:, n * TT:(n + 1) * TT].astype(f32)
        if pin is not None:
            x = jnp.concatenate([jnp.where(false_row[0], pin, x[0:8]), x[8:]], axis=0)
        mu = jnp.mean(x, axis=0, keepdims=True)
        xc = x - mu
        var = jnp.mean(xc * xc, axis=0, keepdims=True)
        if not false_row:
            false_row.append(var < -1.0)
        return (xc * jax.lax.rsqrt(var + EPS)).astype(bf16)

    row4 = jax.lax.broadcasted_iota(jnp.int32, (HP - DH, TT), 0)
    z4 = jnp.zeros((HP - DH, TT), f32)
    one4 = jnp.where(row4 == 0, 1.0, 0.0).astype(f32)

    def qkv_proj(n, xnt, do_q=True, do_kv=True):
        cols = slice(n * TT, (n + 1) * TT)
        r0 = 0 if do_q else D
        r1 = 3 * D if do_kv else D
        qkv = jnp.dot(_up(wt_p[r0 // 2:r1 // 2, :]), xnt, preferred_element_type=f32)
        if do_q:
            for h in range(H):
                q = qkv[DH * h:DH * (h + 1)] * QSCALE
                qt_p[h, :, cols] = _pk(jnp.concatenate([q, z4], axis=0).astype(bf16))
        if do_kv:
            ko = D - r0
            vo = 2 * D - r0
            if n == 0:
                kt32[...] = qkv[ko:ko + D]
            else:
                for g in range(G):
                    parts = []
                    for j in range(4):
                        h = 4 * g + j
                        parts += [qkv[ko + DH * h:ko + DH * (h + 1)], z4]
                    k_p[g, n * TT // 2:(n + 1) * TT // 2, :] = _pk(
                        jnp.concatenate(parts, axis=0).astype(bf16).T)
            for h in range(H):
                v = qkv[vo + DH * h:vo + DH * (h + 1)]
                vt_p[h, :, cols] = _pk(jnp.concatenate([v, one4], axis=0).astype(bf16))
        late = (r1 - r0) * 5 // 64 * 8
        return qkv[0:8], qkv[late:late + 8]

    def kb_gen(lo, hi, pin):
        for r in range(lo, hi):
            row8 = jnp.where(false_row[0], pin, jnp.broadcast_to(kt32[r:r + 1, :], (8, TT)))
            kb = jnp.concatenate([row8] * (TT // 8), axis=0).astype(bf16).T
            kb_ref[r] = kb.astype(f32)

    ntile = S // TT
    n0 = X0 // TT
    cp_x0.wait()
    xnts = [layernorm(n) for n in range(n0)]
    cp_wa.wait()
    wt_p[0:WA // 2, :] = _pk(wqkv_v[:, 0:WA].T)
    for n in range(n0 - 1):
        qkv_proj(n, xnts[n], do_kv=False)
    for n in range(n0):
        store_xn(n, xnts[n])
    cp_wb.wait()
    cp_wo.start()
    cp_w1.start()
    cp_w3.start()
    cp_w2.start()
    wt_p[WA // 2:3 * D // 2, :] = _pk(wqkv_v[:, WA:3 * D].T)
    qkv_proj(n0 - 1, xnts[n0 - 1], do_kv=False)
    nkb = ntile - 1
    pins = []
    for n in range(ntile):
        if n == n0 - 1:
            cp_x1.wait()
            cp_wo.wait()
        if n < n0:
            xnt = xnts[n]
        else:
            xnt = layernorm(n, pins[n - 2][1])
            store_xn(n, xnt)
        pins.append(qkv_proj(n, xnt, do_q=(n >= n0)))
        if n >= 1:
            kb_gen((n - 1) * D // nkb, n * D // nkb, pins[n][0])
        if n == ntile - 2:
            wo32 = wo_v[...].astype(f32)
            z4w = jnp.zeros((HP - DH, D), f32)
            parts = []
            for h in range(H):
                parts += [wo32[DH * h:DH * (h + 1), :], z4w]
            wot_p[...] = _pk(jnp.concatenate(parts, axis=0).astype(bf16).T)
    cp_w1.wait()
    cp_w3.wait()
    cp_w2.wait()

    def out_copy(b):
        r0 = pl.multiple_of(b * BQ, BQ)
        return pltpu.make_async_copy(out_v.at[:, pl.ds(r0, BQ)],
                                     out_hbm.at[:, pl.ds(r0, BQ)], sems.at[5])

    def body(b, carry):
        q0 = pl.multiple_of(b * BQ, BQ)
        zs = pl.multiple_of(z_ref[0], 8)
        zl = pl.multiple_of(z_ref[1], 8)
        never = jax.lax.broadcasted_iota(jnp.int32, (16, QT), 1) < z_ref[0]

        def stage_q(h):
            qs_ref[HP * h:HP * (h + 1), :] = _up(qt_p[h, :, pl.ds(q0, BQ)]).astype(f32)

        for h in reversed(range(H - Q_AHEAD, H)):
            stage_q(h)
        xc_p[...] = xn_p[pl.ds(pl.multiple_of(b * (BQ // 2), BQ // 2), BQ // 2), :]

        def q_weights(it):
            g, t = it // NT, it % NT
            cols = []
            for j in range(4):
                qj = _up(qt_p[4 * g + j, :, pl.ds(q0 + t * QT, QT)])
                parts = []
                if j > 0:
                    parts.append(jnp.zeros((HP * j, QT), bf16))
                parts.append(qj)
                if j < 3:
                    parts.append(jnp.zeros((HP * (3 - j), QT), bf16))
                cols.append(jnp.concatenate(parts, axis=0))
            return jnp.concatenate(cols, axis=1)

        def qk_chunk(it, c, qm, mrun):
            sbuf = s_a if it % 2 == 0 else s_b
            s = jnp.dot(_up(k_p[it // NT, c * C // 2:(c + 1) * C // 2, :]), qm,
                        preferred_element_type=f32)
            sbuf[pl.ds(zs + c * C, C), :] = s
            mc = jnp.max(s.reshape(C // 8, 8, W), axis=0)
            return mc if mrun is None else jnp.maximum(mrun, mc)

        def vpu_scores():
            chain = None
            pending = []
            for t in reversed(range(NT)):
                cs = slice(t * QT, (t + 1) * QT)
                for h in reversed(range(H)):
                    qr = [qs_ref[HP * h + d:HP * h + d + 1, cs] for d in range(DH)]
                    vmax = None
                    for r in range(C // 16):
                        acc = None
                        for d in range(0, DH, 4):
                            p0, p1, p2, p3 = [
                                kb_ref[DH * h + d + i, r * 16:(r + 1) * 16, :] * qr[d + i]
                                for i in range(4)]
                            if acc is not None:
                                acc = acc + p0
                            elif chain is None:
                                acc = p0
                            else:
                                acc = jax.lax.select(never, chain, p0)
                            acc = (acc + p1) + (p2 + p3)
                        chain = acc
                        vmax = acc if vmax is None else jnp.maximum(vmax, acc)
                        pending.append((QR + h * SVR + r * 16, cs, acc))
                    pending.append((QR + h * SVR + C, cs, jnp.maximum(vmax[0:8], vmax[8:16])))
                    if t == NT - 1 and h >= Q_AHEAD:
                        stage_q(h - Q_AHEAD)
                    while len(pending) > 2:
                        row, cols, val = pending.pop(0)
                        qs_ref[pl.ds(zs + row, val.shape[0]), cols] = val
            for row, cols, val in pending:
                qs_ref[pl.ds(zs + row, val.shape[0]), cols] = val

        def final_max(it, mrun):
            g, t = it // NT, it % NT
            vm = jnp.concatenate(
                [qs_ref[QR + (4 * g + j) * SVR + C:QR + (4 * g + j + 1) * SVR, t * QT:(t + 1) * QT]
                 for j in range(4)], axis=1)
            return jnp.max(jnp.maximum(mrun, vm), axis=0, keepdims=True)

        def pv_chunk(it, c, m, o):
            g, t = it // NT, it % NT
            sbuf = s_a if it % 2 == 0 else s_b
            oc = []
            for j in range(4):
                cs = slice(j * QT, (j + 1) * QT)
                if c == 0:
                    r0 = QR + (4 * g + j) * SVR
                    s = qs_ref[r0:r0 + C, t * QT:(t + 1) * QT]
                else:
                    s = sbuf[pl.ds(zl + c * C, C), cs]
                p = jnp.exp2(s - m[:, cs]).astype(bf16)
                oc.append(jnp.dot(_up(vt_p[4 * g + j, :, c * C:(c + 1) * C]), p,
                                  preferred_element_type=f32))
            return oc if o is None else [a + e for a, e in zip(o, oc)]

        def ffn_gate(c, r0=0, n=BQ):
            xn = _up(xc_p[r0 // 2:(r0 + n) // 2, :])
            gate = jnp.dot(xn, w1_v[:, c * FC:(c + 1) * FC], preferred_element_type=f32)
            hg = 0.5 * gate
            return hg * jnp.tanh(hg) + hg

        def ffn_up(c, act, r0=0, n=BQ):
            xn = _up(xc_p[r0 // 2:(r0 + n) // 2, :])
            cols = slice(c * FC, (c + 1) * FC)
            up = jnp.dot(xn, w3_v[:, cols], preferred_element_type=f32)
            h_p[r0 // 2:(r0 + n) // 2, cols] = _pk((act * up).astype(bf16))

        def ffn_down(lo, hi):
            return jax.lax.dot_general(w2_v[:, lo:hi], _up(h_p[:, lo:hi]), _NT_DIMS,
                                       preferred_element_type=f32)

        def wo_proj(lo, hi, r0=0, n=D):
            ot = _up(ot_p[lo:hi].reshape((hi - lo) * HP // 2, BQ))
            return jnp.dot(_up(wot_p[r0 // 2:(r0 + n) // 2, lo * HP:hi * HP]), ot,
                           preferred_element_type=f32)

        vpu_scores()
        mrun = None
        qm = q_weights(0)
        dn = None
        nq = 1
        for i in range(NHEAD // 2 + 1):
            if i < NHEAD // 2:
                for c in (2 * i, 2 * i + 1):
                    ffn_up(c, ffn_gate(c))
            for c in range(nq, nq + QK0_SPREAD[i]):
                mrun = qk_chunk(0, c, qm, mrun)
            nq += QK0_SPREAD[i]
            if i > 0:
                part = ffn_down(2 * (i - 1) * FC, 2 * i * FC)
                dn = part if dn is None else dn + part
        assert nq == NC
        acc_ref[pl.ds(zs, D), :] = dn
        m = final_max(0, mrun)

        acc = None
        for it in range(NITEM):
            mrun = None
            o = None
            if it + 1 < NITEM:
                qm = q_weights(it + 1)
                nslot = NC - LAG
                pv = 0
                for c in range(1, NC):
                    mrun = qk_chunk(it + 1, c, qm, mrun)
                    if c >= LAG:
                        while pv < ((c - LAG + 1) * (NC - 1)) // nslot:
                            o = pv_chunk(it, pv, m, o)
                            pv += 1
                o = pv_chunk(it, NC - 1, m, o)
                m = final_max(it + 1, mrun)
            else:
                fill = []
                for c in range(NHEAD, NFFN):
                    for i in range(NT):
                        fill.append(("gate", c, i))
                        fill.append(("up", c, i))
                fill += [("wo", 0, i) for i in range(NWS)]
                accs = []
                act = None
                for c in range(NC):
                    for k, (kind, fc, i) in enumerate(fill):
                        if k * NC // len(fill) != c:
                            continue
                        if kind == "gate":
                            act = ffn_gate(fc, i * QT, QT)
                        elif kind == "up":
                            ffn_up(fc, act, i * QT, QT)
                        else:
                            r0, n = i * D // NWS, D // NWS
                            accs.append(acc_ref[pl.ds(zl + r0, n), :] + wo_proj(0, H // 2, r0, n))
                    o = pv_chunk(it, c, m, o)
                acc = jnp.concatenate(accs, axis=0) + ffn_down(NHEAD * FC, F)
            g, t = it // NT, it % NT
            for j in range(4):
                inv = 1.0 / o[j][DH:DH + 1, :]
                ot_p[4 * g + j, :, t * QT:(t + 1) * QT] = _pk((o[j] * inv).astype(bf16))
        acc = acc + x_v[:, pl.ds(q0, BQ)].astype(f32)
        acc = acc + wo_proj(H // 2, H)
        out_v[:, pl.ds(q0, BQ)] = acc.astype(bf16)
        out_copy(b).start()
        return carry

    jax.lax.fori_loop(0, S // BQ, body, 0)
    for b in range(S // BQ):
        out_copy(b).wait()


@jax.jit
def pallas_parallel_sum__softmax_full_mha__glu_gated_swiglu__prompt_kernel(
    A_x: jax.Array,
    A_wqkv: jax.Array,
    A_wo: jax.Array,
    B_x: jax.Array,
    B_w1: jax.Array,
    B_w3: jax.Array,
    B_w2: jax.Array,
):
    del B_x
    xt = A_x.reshape(S, D).T
    hbm_spec = pl.BlockSpec(memory_space=pltpu.MemorySpace.HBM)
    out = pl.pallas_call(
        _kernel,
        out_shape=jax.ShapeDtypeStruct((D, S), bf16),
        in_specs=[hbm_spec] * 6,
        out_specs=hbm_spec,
        scratch_shapes=[
            pltpu.VMEM((D, S), bf16),
            pltpu.VMEM((D, 3 * D), bf16),
            pltpu.VMEM((D, D), bf16),
            pltpu.VMEM((D, F), bf16),
            pltpu.VMEM((D, F), bf16),
            pltpu.VMEM((D, F), bf16),
            pltpu.VMEM((S // 2, D), u32),
            pltpu.VMEM((BQ // 2, D), u32),
            pltpu.VMEM((3 * D // 2, D), u32),
            pltpu.VMEM((D // 2, H * HP), u32),
            pltpu.VMEM((D, TT), f32),
            pltpu.VMEM((G, S // 2, 128), u32),
            pltpu.VMEM((H, HP // 2, S), u32),
            pltpu.VMEM((QR + H * SVR, BQ), f32),
            pltpu.VMEM((H, HP // 2, S), u32),
            pltpu.VMEM((D, C, 128), f32),
            pltpu.VMEM((S, W), f32),
            pltpu.VMEM((S, W), f32),
            pltpu.VMEM((H, HP // 2, BQ), u32),
            pltpu.VMEM((BQ // 2, F), u32),
            pltpu.VMEM((D, BQ), f32),
            pltpu.VMEM((D, S), bf16),
            pltpu.SMEM((2,), jnp.int32),
            pltpu.SemaphoreType.DMA((6,)),
        ],
        compiler_params=pltpu.CompilerParams(vmem_limit_bytes=100 * 1024 * 1024),
    )(xt, A_wqkv, A_wo, B_w1, B_w3, B_w2.T)
    return out.T.reshape(1, S, D)
```

```python
import math

import jax
import jax.numpy as jnp
import jax.experimental.pallas as pl
import jax.experimental.pallas.tpu as pltpu

S = 2048
D = 448
H = 16
DH = D // H
F = 1792
G = 4
HP = 32
QT = 128
W = 4 * QT
BQ = 256
NT = BQ // QT
NITEM = NT * G
C = 128
NC = S // C
LAG = 3
TT = 128
FC = 128
NFFN = F // FC
NTAIL = 2
NHEAD = NFFN - NTAIL
QK0_SPREAD = (1, 2, 2, 2, 2, 3, 3)
Q_AHEAD = 3
NWS = 7
GB = 8
X0 = 512
WA = 512
QR = H * HP
SVR = C + 8
EPS = 1e-5
QSCALE = (DH ** -0.5) * math.log2(math.e)

_NT_DIMS = (((1,), (1,)), ((), ()))
f32 = jnp.float32
bf16 = jnp.bfloat16
u32 = jnp.uint32


def _pk(x):
    return pltpu.bitcast(x, u32)


def _up(x):
    return pltpu.bitcast(x, bf16)


def _kernel(x_hbm, wqkv_hbm, wo_hbm, w1_hbm, w3_hbm, w2_hbm, out_hbm,
            x_v, wqkv_v, wo_v, w1_v, w3_v, w2_v,
            xn_p, xc_p, wt_p, wot_p, kt32,
            k_p, qt_p, qs_ref, vt_p, kb_ref, s_a, s_b,
            ot_p, h_p, acc_ref, out_v, z_ref, sems):
    def cols_copy(src, dst, lo, n, sem):
        return pltpu.make_async_copy(src.at[:, pl.ds(lo, n)], dst.at[:, pl.ds(lo, n)], sem)

    cp_x0 = cols_copy(x_hbm, x_v, 0, X0, sems.at[0])
    cp_wa = cols_copy(wqkv_hbm, wqkv_v, 0, WA, sems.at[1])
    cp_wb = cols_copy(wqkv_hbm, wqkv_v, WA, 3 * D - WA, sems.at[2])
    cp_x1 = cols_copy(x_hbm, x_v, X0, S - X0, sems.at[3])
    cp_wo = pltpu.make_async_copy(wo_hbm, wo_v, sems.at[3])
    cp_w1 = pltpu.make_async_copy(w1_hbm, w1_v, sems.at[4])
    cp_w3 = pltpu.make_async_copy(w3_hbm, w3_v, sems.at[4])
    cp_w2 = pltpu.make_async_copy(w2_hbm, w2_v, sems.at[4])
    cp_x0.start()
    cp_wa.start()
    cp_wb.start()
    cp_x1.start()
    z_ref[0] = 0
    z_ref[1] = 0

    false_row = []

    def store_xn(n, xnt):
        xn_p[n * TT // 2:(n + 1) * TT // 2, :] = _pk(xnt.T)

    def layernorm(n, pin=None):
        x = x_v[:, n * TT:(n + 1) * TT].astype(f32)
        if pin is not None:
            x = jnp.concatenate([jnp.where(false_row[0], pin, x[0:8]), x[8:]], axis=0)
        mu = jnp.mean(x, axis=0, keepdims=True)
        xc = x - mu
        var = jnp.mean(xc * xc, axis=0, keepdims=True)
        if not false_row:
            false_row.append(var < -1.0)
        return (xc * jax.lax.rsqrt(var + EPS)).astype(bf16)

    row4 = jax.lax.broadcasted_iota(jnp.int32, (HP - DH, TT), 0)
    z4 = jnp.zeros((HP - DH, TT), f32)
    one4 = jnp.where(row4 == 0, 1.0, 0.0).astype(f32)

    def qkv_proj(n, xnt, do_q=True, do_kv=True):
        cols = slice(n * TT, (n + 1) * TT)
        r0 = 0 if do_q else D
        r1 = 3 * D if do_kv else D
        qkv = jnp.dot(_up(wt_p[r0 // 2:r1 // 2, :]), xnt, preferred_element_type=f32)
        if do_q:
            for h in range(H):
                q = qkv[DH * h:DH * (h + 1)] * QSCALE
                qt_p[h, :, cols] = _pk(jnp.concatenate([q, z4], axis=0).astype(bf16))
        if do_kv:
            ko = D - r0
            vo = 2 * D - r0
            if n == 0:
                kt32[...] = qkv[ko:ko + D]
            else:
                for g in range(G):
                    parts = []
                    for j in range(4):
                        h = 4 * g + j
                        parts += [qkv[ko + DH * h:ko + DH * (h + 1)], z4]
                    k_p[g, n * TT // 2:(n + 1) * TT // 2, :] = _pk(
                        jnp.concatenate(parts, axis=0).astype(bf16).T)
            for h in range(H):
                v = qkv[vo + DH * h:vo + DH * (h + 1)]
                vt_p[h, :, cols] = _pk(jnp.concatenate([v, one4], axis=0).astype(bf16))
        late = (r1 - r0) * 5 // 64 * 8
        return qkv[0:8], qkv[late:late + 8]

    def kb_gen(lo, hi, pin):
        for r in range(lo, hi):
            row8 = jnp.where(false_row[0], pin, jnp.broadcast_to(kt32[r:r + 1, :], (8, TT)))
            kb = jnp.concatenate([row8] * (TT // 8), axis=0).astype(bf16).T
            kb_ref[r] = kb.astype(f32)

    ntile = S // TT
    n0 = X0 // TT
    cp_x0.wait()
    xnts = [layernorm(n) for n in range(n0)]
    cp_wa.wait()
    wt_p[0:WA // 2, :] = _pk(wqkv_v[:, 0:WA].T)
    for n in range(n0 - 1):
        qkv_proj(n, xnts[n], do_kv=False)
    for n in range(n0):
        store_xn(n, xnts[n])
    cp_wb.wait()
    cp_wo.start()
    cp_w1.start()
    cp_w3.start()
    cp_w2.start()
    wt_p[WA // 2:3 * D // 2, :] = _pk(wqkv_v[:, WA:3 * D].T)
    qkv_proj(n0 - 1, xnts[n0 - 1], do_kv=False)
    nkb = ntile - 1
    pins = []
    for n in range(ntile):
        if n == n0 - 1:
            cp_x1.wait()
            cp_wo.wait()
        if n < n0:
            xnt = xnts[n]
        else:
            xnt = layernorm(n, pins[n - 2][1])
            store_xn(n, xnt)
        pins.append(qkv_proj(n, xnt, do_q=(n >= n0)))
        if n >= 1:
            kb_gen((n - 1) * D // nkb, n * D // nkb, pins[n][0])
        if n == ntile - 2:
            wo32 = wo_v[...].astype(f32)
            z4w = jnp.zeros((HP - DH, D), f32)
            parts = []
            for h in range(H):
                parts += [wo32[DH * h:DH * (h + 1), :], z4w]
            wot_p[...] = _pk(jnp.concatenate(parts, axis=0).astype(bf16).T)
    cp_w1.wait()
    cp_w3.wait()
    cp_w2.wait()

    def out_copy(b, t):
        r0 = pl.multiple_of(b * BQ + t * QT, QT)
        return pltpu.make_async_copy(out_v.at[:, pl.ds(r0, QT)],
                                     out_hbm.at[:, pl.ds(r0, QT)], sems.at[5])

    def body(b, carry):
        q0 = pl.multiple_of(b * BQ, BQ)
        zs = pl.multiple_of(z_ref[0], 8)
        zl = pl.multiple_of(z_ref[1], 8)
        never = jax.lax.broadcasted_iota(jnp.int32, (16, QT), 1) < z_ref[0]

        def stage_q(h):
            qs_ref[HP * h:HP * (h + 1), :] = _up(qt_p[h, :, pl.ds(q0, BQ)]).astype(f32)

        for h in reversed(range(H - Q_AHEAD, H)):
            stage_q(h)
        xc_p[...] = xn_p[pl.ds(pl.multiple_of(b * (BQ // 2), BQ // 2), BQ // 2), :]

        def q_weights(it):
            g, t = it // NT, it % NT
            cols = []
            for j in range(4):
                qj = _up(qt_p[4 * g + j, :, pl.ds(q0 + t * QT, QT)])
                parts = []
                if j > 0:
                    parts.append(jnp.zeros((HP * j, QT), bf16))
                parts.append(qj)
                if j < 3:
                    parts.append(jnp.zeros((HP * (3 - j), QT), bf16))
                cols.append(jnp.concatenate(parts, axis=0))
            return jnp.concatenate(cols, axis=1)

        def qk_chunk(it, c, qm, mrun):
            sbuf = s_a if it % 2 == 0 else s_b
            s = jnp.dot(_up(k_p[it // NT, c * C // 2:(c + 1) * C // 2, :]), qm,
                        preferred_element_type=f32)
            sbuf[pl.ds(zs + c * C, C), :] = s
            mc = jnp.max(s.reshape(C // 8, 8, W), axis=0)
            return mc if mrun is None else jnp.maximum(mrun, mc)

        def vpu_scores():
            chain = None
            pending = []
            for t in reversed(range(NT)):
                cs = slice(t * QT, (t + 1) * QT)
                for h in reversed(range(H)):
                    qr = [qs_ref[HP * h + d:HP * h + d + 1, cs] for d in range(DH)]
                    vmax = None
                    for r in range(C // 16):
                        acc = None
                        for d in range(0, DH, 4):
                            if d % GB == 0:
                                nb = min(GB, DH - d)
                                kb = kb_ref[DH * h + d:DH * h + d + nb, r * 16:(r + 1) * 16, :]
                                kb = kb.reshape(nb * 16, QT)
                            p0, p1, p2, p3 = [
                                kb[(d % GB + i) * 16:(d % GB + i + 1) * 16] * qr[d + i]
                                for i in range(4)]
                            if acc is not None:
                                acc = acc + p0
                            elif chain is None:
                                acc = p0
                            else:
                                acc = jax.lax.select(never, chain, p0)
                            acc = (acc + p1) + (p2 + p3)
                        chain = acc
                        vmax = acc if vmax is None else jnp.maximum(vmax, acc)
                        pending.append((QR + h * SVR + r * 16, cs, acc))
                    pending.append((QR + h * SVR + C, cs, jnp.maximum(vmax[0:8], vmax[8:16])))
                    if t == NT - 1 and h >= Q_AHEAD:
                        stage_q(h - Q_AHEAD)
                    while len(pending) > 2:
                        row, cols, val = pending.pop(0)
                        qs_ref[pl.ds(zs + row, val.shape[0]), cols] = val
            for row, cols, val in pending:
                qs_ref[pl.ds(zs + row, val.shape[0]), cols] = val

        def final_max(it, mrun):
            g, t = it // NT, it % NT
            vm = jnp.concatenate(
                [qs_ref[QR + (4 * g + j) * SVR + C:QR + (4 * g + j + 1) * SVR, t * QT:(t + 1) * QT]
                 for j in range(4)], axis=1)
            return jnp.max(jnp.maximum(mrun, vm), axis=0, keepdims=True)

        def pv_chunk(it, c, m, o):
            g, t = it // NT, it % NT
            sbuf = s_a if it % 2 == 0 else s_b
            oc = []
            for j in range(4):
                cs = slice(j * QT, (j + 1) * QT)
                if c == 0:
                    r0 = QR + (4 * g + j) * SVR
                    s = qs_ref[r0:r0 + C, t * QT:(t + 1) * QT]
                else:
                    s = sbuf[pl.ds(zl + c * C, C), cs]
                p = jnp.exp2(s - m[:, cs]).astype(bf16)
                oc.append(jnp.dot(_up(vt_p[4 * g + j, :, c * C:(c + 1) * C]), p,
                                  preferred_element_type=f32))
            return oc if o is None else [a + e for a, e in zip(o, oc)]

        def ffn_gate(c, r0=0, n=BQ):
            xn = _up(xc_p[r0 // 2:(r0 + n) // 2, :])
            gate = jnp.dot(xn, w1_v[:, c * FC:(c + 1) * FC], preferred_element_type=f32)
            hg = 0.5 * gate
            return hg * jnp.tanh(hg) + hg

        def ffn_up(c, act, r0=0, n=BQ):
            xn = _up(xc_p[r0 // 2:(r0 + n) // 2, :])
            cols = slice(c * FC, (c + 1) * FC)
            up = jnp.dot(xn, w3_v[:, cols], preferred_element_type=f32)
            h_p[r0 // 2:(r0 + n) // 2, cols] = _pk((act * up).astype(bf16))

        def ffn_down(lo, hi):
            return jax.lax.dot_general(w2_v[:, lo:hi], _up(h_p[:, lo:hi]), _NT_DIMS,
                                       preferred_element_type=f32)

        def wo_proj(t, r0=0, n=D):
            ot = _up(ot_p[:, :, t * QT:(t + 1) * QT].reshape(H * HP // 2, QT))
            return jnp.dot(_up(wot_p[r0 // 2:(r0 + n) // 2, :]), ot, preferred_element_type=f32)

        vpu_scores()
        mrun = None
        qm = q_weights(0)
        dn = None
        nq = 1
        for i in range(NHEAD // 2 + 1):
            if i < NHEAD // 2:
                for c in (2 * i, 2 * i + 1):
                    ffn_up(c, ffn_gate(c))
            for c in range(nq, nq + QK0_SPREAD[i]):
                mrun = qk_chunk(0, c, qm, mrun)
            nq += QK0_SPREAD[i]
            if i > 0:
                part = ffn_down(2 * (i - 1) * FC, 2 * i * FC)
                dn = part if dn is None else dn + part
        assert nq == NC
        acc_ref[pl.ds(zs, D), :] = dn
        m = final_max(0, mrun)

        acc = None
        for it in range(NITEM):
            mrun = None
            o = None
            if it + 1 < NITEM:
                qm = q_weights(it + 1)
                nslot = NC - LAG
                pv = 0
                for c in range(1, NC):
                    mrun = qk_chunk(it + 1, c, qm, mrun)
                    if c >= LAG:
                        while pv < ((c - LAG + 1) * (NC - 1)) // nslot:
                            o = pv_chunk(it, pv, m, o)
                            pv += 1
                o = pv_chunk(it, NC - 1, m, o)
                m = final_max(it + 1, mrun)
            else:
                fill = []
                for c in range(NHEAD, NFFN):
                    for i in range(NT):
                        fill.append(("gate", c, i))
                        fill.append(("up", c, i))
                fill += [("wo", 0, i) for i in range(NWS)]
                accs = []
                act = None
                for c in range(NC):
                    for k, (kind, fc, i) in enumerate(fill):
                        if k * NC // len(fill) != c:
                            continue
                        if kind == "gate":
                            act = ffn_gate(fc, i * QT, QT)
                        elif kind == "up":
                            ffn_up(fc, act, i * QT, QT)
                        else:
                            r0, n = i * D // NWS, D // NWS
                            accs.append(acc_ref[pl.ds(zl + r0, n), 0:QT] + wo_proj(0, r0, n))
                    o = pv_chunk(it, c, m, o)
                acc = ffn_down(NHEAD * FC, F) + x_v[:, pl.ds(q0, BQ)].astype(f32)
                out_v[:, pl.ds(q0, QT)] = (jnp.concatenate(accs, axis=0) + acc[:, 0:QT]).astype(bf16)
                out_copy(b, 0).start()
            g, t = it // NT, it % NT
            for j in range(4):
                inv = 1.0 / o[j][DH:DH + 1, :]
                ot_p[4 * g + j, :, t * QT:(t + 1) * QT] = _pk((o[j] * inv).astype(bf16))
        acc = (acc[:, QT:BQ] + acc_ref[pl.ds(zl, D), QT:BQ]) + wo_proj(1)
        out_v[:, pl.ds(pl.multiple_of(q0 + QT, QT), QT)] = acc.astype(bf16)
        out_copy(b, 1).start()
        return carry

    jax.lax.fori_loop(0, S // BQ, body, 0)
    for b in range(S // BQ):
        for t in range(NT):
            out_copy(b, t).wait()


@jax.jit
def pallas_parallel_sum__softmax_full_mha__glu_gated_swiglu__prompt_kernel(
    A_x: jax.Array,
    A_wqkv: jax.Array,
    A_wo: jax.Array,
    B_x: jax.Array,
    B_w1: jax.Array,
    B_w3: jax.Array,
    B_w2: jax.Array,
):
    del B_x
    xt = A_x.reshape(S, D).T
    hbm_spec = pl.BlockSpec(memory_space=pltpu.MemorySpace.HBM)
    out = pl.pallas_call(
        _kernel,
        out_shape=jax.ShapeDtypeStruct((D, S), bf16),
        in_specs=[hbm_spec] * 6,
        out_specs=hbm_spec,
        scratch_shapes=[
            pltpu.VMEM((D, S), bf16),
            pltpu.VMEM((D, 3 * D), bf16),
            pltpu.VMEM((D, D), bf16),
            pltpu.VMEM((D, F), bf16),
            pltpu.VMEM((D, F), bf16),
            pltpu.VMEM((D, F), bf16),
            pltpu.VMEM((S // 2, D), u32),
            pltpu.VMEM((BQ // 2, D), u32),
            pltpu.VMEM((3 * D // 2, D), u32),
            pltpu.VMEM((D // 2, H * HP), u32),
            pltpu.VMEM((D, TT), f32),
            pltpu.VMEM((G, S // 2, 128), u32),
            pltpu.VMEM((H, HP // 2, S), u32),
            pltpu.VMEM((QR + H * SVR, BQ), f32),
            pltpu.VMEM((H, HP // 2, S), u32),
            pltpu.VMEM((D, C, 128), f32),
            pltpu.VMEM((S, W), f32),
            pltpu.VMEM((S, W), f32),
            pltpu.VMEM((H, HP // 2, BQ), u32),
            pltpu.VMEM((BQ // 2, F), u32),
            pltpu.VMEM((D, BQ), f32),
            pltpu.VMEM((D, S), bf16),
            pltpu.SMEM((2,), jnp.int32),
            pltpu.SemaphoreType.DMA((6,)),
        ],
        compiler_params=pltpu.CompilerParams(vmem_limit_bytes=100 * 1024 * 1024),
    )(xt, A_wqkv, A_wo, B_w1, B_w3, B_w2.T)
    return out.T.reshape(1, S, D)
```

```python
import math

import jax
import jax.numpy as jnp
import jax.experimental.pallas as pl
import jax.experimental.pallas.tpu as pltpu

S = 2048
D = 448
H = 16
DH = D // H
F = 1792
G = 4
HP = 32
QT = 128
W = 4 * QT
BQ = 256
NT = BQ // QT
NITEM = NT * G
C = 128
NC = S // C
EX = 48
NOFF = C + EX
NBUF = 5
TT = 128
FC = 128
NFFN = F // FC
NHEAD = NFFN - 2
X0 = 512
WA = 512
QR = H * HP
SVR = NOFF + 8
EPS = 1e-5
QSCALE = (DH ** -0.5) * math.log2(math.e)

L0 = 33
LAG = 3
HB = 2
TPV = 18
MG = 2
QK_SPREAD = (1, 2, 2, 2, 2, 3, 3)
Q_AHEAD = 3
NWS = 7
GB = 8
FAST_FROM = 88
KB_WEIGHTS = (2, 2, 2) + (3,) * 12

_NT_DIMS = (((1,), (1,)), ((), ()))
f32 = jnp.float32
bf16 = jnp.bfloat16
u32 = jnp.uint32


def _ex_lo(g):
    return 0 if g < G // 2 else C - EX


def _schedule():
    nq = NC - 1
    nqk = (NITEM - 1) * nq
    npv = NITEM * NC - TPV
    pos = []
    for p in range(npv):
        q = L0 + (p * (nqk - L0)) // (npv - 1)
        pos.append(max(q, min(nqk, (p // NC) * nq + LAG), pos[-1] if pos else 0))
    for it in range(NITEM):
        a, e = it * NC, min(npv, (it + 1) * NC)
        if a >= npv:
            break
        nxt = pos[e] if e < npv else nqk
        if e < npv and pos[e] == (it + 1) * nq + LAG:
            nxt = pos[e] - LAG
        for p in range(a, e):
            pos[p] = pos[a] + ((p - a) * (nxt - pos[a])) // max(1, e - a - 1)
    pos = [q + nq for q in pos]
    ntot = NITEM * nq
    slots = [None] * ntot
    for it in range(NITEM):
        end = min(pos[it * NC] - LAG, ntot) if it * NC < npv else ntot
        for i in range(HB):
            slots[end - HB + i] = (it, NC - HB + i)
    rest = iter([(it, c) for it in range(NITEM) for c in range(1, NC - HB)])
    slots = [s if s is not None else next(rest) for s in slots]
    seen = {}
    for k, (it, c) in enumerate(slots):
        assert c == seen.get(it, 0) + 1
        seen[it] = c
        if c == 1 and it >= NBUF:
            assert pos[(it - NBUF + 1) * NC - 1] <= k
        if c == NC - 1 and it * NC < npv:
            assert k < pos[it * NC]
    return slots, pos


_SLOTS, _PV_POS = _schedule()


def _pk(x):
    return pltpu.bitcast(x, u32)


def _up(x):
    return pltpu.bitcast(x, bf16)


def _kernel(x_hbm, wqkv_hbm, wo_hbm, w1_hbm, w3_hbm, w2_hbm, out_hbm,
            x_v, wqkv_v, wo_v, w1_v, w3_v, w2_v,
            xn_p, xc_p, wt_p, wot_p, kt32, kx32,
            k_p, qt_p, qs_ref, vt_p, kb_ref, kbx_ref,
            ot_p, h_p, acc_ref, out_v, z_ref, sems, s_all):
    def cols_copy(src, dst, lo, n, sem):
        return pltpu.make_async_copy(src.at[:, pl.ds(lo, n)], dst.at[:, pl.ds(lo, n)], sem)

    cp_x0 = cols_copy(x_hbm, x_v, 0, X0, sems.at[0])
    cp_wa = cols_copy(wqkv_hbm, wqkv_v, 0, WA, sems.at[1])
    cp_wb = cols_copy(wqkv_hbm, wqkv_v, WA, 3 * D - WA, sems.at[2])
    cp_x1 = cols_copy(x_hbm, x_v, X0, S - X0, sems.at[3])
    cp_wo = pltpu.make_async_copy(wo_hbm, wo_v, sems.at[3])
    cp_w1 = pltpu.make_async_copy(w1_hbm, w1_v, sems.at[4])
    cp_w3 = pltpu.make_async_copy(w3_hbm, w3_v, sems.at[4])
    cp_w2 = pltpu.make_async_copy(w2_hbm, w2_v, sems.at[4])
    cp_x0.start()
    cp_wa.start()
    cp_wb.start()
    cp_x1.start()
    z_ref[0] = 0
    z_ref[1] = 0
    s_all[0, 0:16, 0:QT] = jnp.zeros((16, QT), f32)

    false_row = []

    def store_xn(n, xnt):
        xn_p[n * TT // 2:(n + 1) * TT // 2, :] = _pk(xnt.T)

    def layernorm(n, pin=None):
        x = x_v[:, n * TT:(n + 1) * TT].astype(f32)
        if pin is not None:
            x = jnp.concatenate([jnp.where(false_row[0], pin, x[0:8]), x[8:]], axis=0)
        mu = jnp.mean(x, axis=0, keepdims=True)
        xc = x - mu
        var = jnp.mean(xc * xc, axis=0, keepdims=True)
        if not false_row:
            false_row.append(var < -1.0)
        return (xc * jax.lax.rsqrt(var + EPS)).astype(bf16)

    row4 = jax.lax.broadcasted_iota(jnp.int32, (HP - DH, TT), 0)
    z4 = jnp.zeros((HP - DH, TT), f32)
    one4 = jnp.where(row4 == 0, 1.0, 0.0).astype(f32)

    def qkv_proj(n, xnt, do_q=True, do_kv=True):
        cols = slice(n * TT, (n + 1) * TT)
        r0 = 0 if do_q else D
        r1 = 3 * D if do_kv else D
        qkv = jnp.dot(_up(wt_p[r0 // 2:r1 // 2, :]), xnt, preferred_element_type=f32)
        if do_q:
            for h in range(H):
                q = qkv[DH * h:DH * (h + 1)] * QSCALE
                qt_p[h, :, cols] = _pk(jnp.concatenate([q, z4], axis=0).astype(bf16))
        if do_kv:
            ko = D - r0
            vo = 2 * D - r0
            if n == 0:
                kt32[...] = qkv[ko:ko + D]
            else:
                if n == 1:
                    lane = jax.lax.broadcasted_iota(jnp.int32, (D // 2, TT), 1)
                    kx32[0:D // 2, :] = jnp.where(lane >= TT // 2, qkv[ko + D // 2:ko + D],
                                                  qkv[ko:ko + D // 2])
                for g in range(G):
                    parts = []
                    for j in range(4):
                        h = 4 * g + j
                        parts += [qkv[ko + DH * h:ko + DH * (h + 1)], z4]
                    k_p[g, n * TT // 2:(n + 1) * TT // 2, :] = _pk(
                        jnp.concatenate(parts, axis=0).astype(bf16).T)
            for h in range(H):
                v = qkv[vo + DH * h:vo + DH * (h + 1)]
                vt_p[h, :, cols] = _pk(jnp.concatenate([v, one4], axis=0).astype(bf16))
        late = (r1 - r0) * 7 // 64 * 8
        return qkv[0:8], qkv[late:late + 8]

    def kb_gen(lo, hi, pin):
        for r in range(lo, hi):
            src = kt32[r:r + 1, :] if r < D else kx32[r - D:r - D + 1, :]
            row8 = jnp.where(false_row[0], pin, jnp.broadcast_to(src, (8, TT)))
            kb = jnp.concatenate([row8] * (TT // 8), axis=0).astype(bf16).T
            if r < D:
                kb_ref[r] = kb.astype(f32)
            else:
                kbx_ref[r - D] = kb[0:EX].astype(f32)
                kbx_ref[r - D + D // 2] = kb[C - EX:C].astype(f32)

    ntile = S // TT
    n0 = X0 // TT
    cp_x0.wait()
    xnts = [layernorm(n) for n in range(n0)]
    cp_wa.wait()
    wt_p[0:WA // 2, :] = _pk(wqkv_v[:, 0:WA].T)
    for n in range(n0 - 1):
        qkv_proj(n, xnts[n], do_kv=False)
    for n in range(n0):
        store_xn(n, xnts[n])
    cp_wb.wait()
    cp_wo.start()
    cp_w1.start()
    cp_w3.start()
    cp_w2.start()
    wt_p[WA // 2:3 * D // 2, :] = _pk(wqkv_v[:, WA:3 * D].T)
    qkv_proj(n0 - 1, xnts[n0 - 1], do_kv=False)
    pins = []
    for n in range(ntile):
        if n == n0 - 1:
            cp_x1.wait()
            cp_wo.wait()
        if n < n0:
            xnt = xnts[n]
        else:
            xnt = layernorm(n, pins[n - 2][1])
            store_xn(n, xnt)
        pins.append(qkv_proj(n, xnt, do_q=(n >= n0)))
        if n >= 1:
            nrow, tot = D + D // 2, sum(KB_WEIGHTS)
            kb_gen(sum(KB_WEIGHTS[:n - 1]) * nrow // tot, sum(KB_WEIGHTS[:n]) * nrow // tot,
                   pins[n][0])
        if n == ntile - 2:
            wo32 = wo_v[...].astype(f32)
            z4w = jnp.zeros((HP - DH, D), f32)
            parts = []
            for h in range(H):
                parts += [wo32[DH * h:DH * (h + 1), :], z4w]
            wot_p[...] = _pk(jnp.concatenate(parts, axis=0).astype(bf16).T)
    cp_w1.wait()
    cp_w3.wait()
    cp_w2.wait()

    def out_copy(b, t):
        r0 = pl.multiple_of(b * BQ + t * QT, QT)
        return pltpu.make_async_copy(out_v.at[:, pl.ds(r0, QT)],
                                     out_hbm.at[:, pl.ds(r0, QT)], sems.at[5])

    def body(b, carry):
        q0 = pl.multiple_of(b * BQ, BQ)
        zs = z_ref[0]
        zl = z_ref[1]
        never = jax.lax.broadcasted_iota(jnp.int32, (16, QT), 1) < zs

        def stage_q(h):
            qs_ref[0, HP * h:HP * (h + 1), :] = _up(qt_p[h, :, pl.ds(q0, BQ)]).astype(f32)

        for h in reversed(range(H - Q_AHEAD, H)):
            stage_q(h)
        xc_p[...] = xn_p[pl.ds(pl.multiple_of(b * (BQ // 2), BQ // 2), BQ // 2), :]

        def vpu_scores():
            chain = s_all[0, 0:16, 0:QT]
            pending = []
            npiece = 0
            for t in reversed(range(NT)):
                cs = slice(t * QT, (t + 1) * QT)
                for h in reversed(range(H)):
                    qr = [qs_ref[0, HP * h + d:HP * h + d + 1, cs] for d in range(DH)]
                    vmax = None
                    for r in range(NOFF // 16):
                        src, rr = (kb_ref, r) if r < C // 16 else (kbx_ref, r - C // 16)
                        late = npiece * 100 >= FAST_FROM * NT * H * (NOFF // 16)
                        acc = None
                        for d in range(0, DH, 4):
                            if d % GB == 0:
                                nb = min(GB, DH - d)
                                kb = src[DH * h + d:DH * h + d + nb, rr * 16:(rr + 1) * 16, :]
                                kb = kb.reshape(nb * 16, QT)
                            p0, p1, p2, p3 = [
                                kb[(d % GB + i) * 16:(d % GB + i + 1) * 16] * qr[d + i]
                                for i in range(4)]
                            if acc is None:
                                acc = jax.lax.select(never, chain, p0)
                                acc = (acc + p1) + (p2 + p3)
                            elif late and d == 12:
                                acc = (acc + (p0 + p1)) + (p2 + p3)
                            else:
                                acc = ((acc + p0) + p1) + (p2 + p3)
                        npiece += 1
                        chain = acc
                        vmax = acc if vmax is None else jnp.maximum(vmax, acc)
                        pending.append((QR + h * SVR + r * 16, cs, acc))
                    pending.append((QR + h * SVR + NOFF, cs, jnp.maximum(vmax[0:8], vmax[8:16])))
                    if t == NT - 1 and h >= Q_AHEAD:
                        stage_q(h - Q_AHEAD)
                    while len(pending) > 2:
                        row, cols, val = pending.pop(0)
                        qs_ref[zs, row:row + val.shape[0], cols] = val
            for row, cols, val in pending:
                qs_ref[zs, row:row + val.shape[0], cols] = val

        def q_weights(it):
            g, t = it // NT, it % NT
            cols = []
            for j in range(4):
                qj = _up(qt_p[4 * g + j, :, pl.ds(q0 + t * QT, QT)])
                parts = []
                if j > 0:
                    parts.append(jnp.zeros((HP * j, QT), bf16))
                parts.append(qj)
                if j < 3:
                    parts.append(jnp.zeros((HP * (3 - j), QT), bf16))
                cols.append(jnp.concatenate(parts, axis=0))
            return jnp.concatenate(cols, axis=1)

        qms, mruns, ms, outs = {}, {}, {}, {}

        def do_qk(k, cnt=1):
            it, c = _SLOTS[k]
            if c == 1:
                qms[it] = q_weights(it)
                lo = C + (EX if _ex_lo(it // NT) == 0 else 0)
                n = C - EX
            else:
                lo, n = c * C, cnt * C
            s = jnp.dot(_up(k_p[it // NT, lo // 2:(lo + n) // 2, :]), qms[it],
                        preferred_element_type=f32)
            s_all[it % NBUF, c * C:c * C + n, :] = s
            mc = jnp.max(s.reshape(n // 8, 8, W), axis=0)
            mruns[it] = mc if c == 1 else jnp.maximum(mruns[it], mc)

        def do_qk_run(k0, k1):
            k = k0
            while k < k1:
                it, c = _SLOTS[k]
                cnt = 1
                while c > 1 and cnt < MG and k + cnt < k1 and _SLOTS[k + cnt] == (it, c + cnt):
                    cnt += 1
                do_qk(k, cnt)
                k += cnt

        def do_pv(p):
            it, c = p // NC, p % NC
            g, t = it // NT, it % NT
            ts = slice(t * QT, (t + 1) * QT)
            if c == 0:
                vm = jnp.concatenate(
                    [qs_ref[0, QR + (4 * g + j) * SVR + NOFF:QR + (4 * g + j + 1) * SVR, ts]
                     for j in range(4)], axis=1)
                ms[it] = jnp.max(jnp.maximum(mruns[it], vm), axis=0, keepdims=True)
            oc = []
            for j in range(4):
                cs = slice(j * QT, (j + 1) * QT)
                r0 = QR + (4 * g + j) * SVR
                if c == 0:
                    s = qs_ref[0, r0:r0 + C, ts]
                elif c == 1:
                    parts = [qs_ref[0, r0 + C:r0 + NOFF, ts], s_all[it % NBUF, C:2 * C - EX, cs]]
                    s = jnp.concatenate(parts if _ex_lo(g) == 0 else parts[::-1], axis=0)
                else:
                    s = s_all[it % NBUF, c * C:(c + 1) * C, cs]
                pr = jnp.exp2(s - ms[it][:, cs]).astype(bf16)
                oc.append(jnp.dot(_up(vt_p[4 * g + j, :, c * C:(c + 1) * C]), pr,
                                  preferred_element_type=f32))
            outs[it] = oc if c == 0 else [a + e for a, e in zip(outs[it], oc)]

        def finish(it):
            g, t = it // NT, it % NT
            for j, o in enumerate(outs[it]):
                inv = 1.0 / o[DH:DH + 1, :]
                ot_p[4 * g + j, :, t * QT:(t + 1) * QT] = _pk((o * inv).astype(bf16))

        def ffn_gate(c, r0=0, n=BQ):
            xn = _up(xc_p[r0 // 2:(r0 + n) // 2, :])
            gate = jnp.dot(xn, w1_v[:, c * FC:(c + 1) * FC], preferred_element_type=f32)
            hg = 0.5 * gate
            return hg * jnp.tanh(hg) + hg

        def ffn_up(c, act, r0=0, n=BQ):
            xn = _up(xc_p[r0 // 2:(r0 + n) // 2, :])
            cols = slice(c * FC, (c + 1) * FC)
            up = jnp.dot(xn, w3_v[:, cols], preferred_element_type=f32)
            h_p[r0 // 2:(r0 + n) // 2, cols] = _pk((act * up).astype(bf16))

        def ffn_down(lo, hi):
            return jax.lax.dot_general(w2_v[:, lo:hi], _up(h_p[:, lo:hi]), _NT_DIMS,
                                       preferred_element_type=f32)

        def wo_proj(t, r0=0, n=D):
            ot = _up(ot_p[:, :, t * QT:(t + 1) * QT].reshape(H * HP // 2, QT))
            return jnp.dot(_up(wot_p[r0 // 2:(r0 + n) // 2, :]), ot, preferred_element_type=f32)

        vpu_scores()
        dn = None
        nq = 0
        for i in range(NHEAD // 2 + 1):
            if i < NHEAD // 2:
                for c in (2 * i, 2 * i + 1):
                    ffn_up(c, ffn_gate(c))
            do_qk_run(nq, nq + QK_SPREAD[i])
            nq += QK_SPREAD[i]
            if i > 0:
                part = ffn_down(2 * (i - 1) * FC, 2 * i * FC)
                dn = part if dn is None else dn + part
        acc_ref[zs] = dn
        do_qk_run(nq, _PV_POS[0])

        pv = 0
        for k in range(_PV_POS[0], len(_SLOTS) + 1):
            while pv < len(_PV_POS) and _PV_POS[pv] <= k:
                do_pv(pv)
                if pv % NC == NC - 1:
                    finish(pv // NC)
                pv += 1
            if k < len(_SLOTS):
                do_qk(k)

        fill = [(kind, c, i) for c in range(NHEAD, NFFN) for i in range(NT)
                for kind in ("gate", "up")]
        fill += [("wo", 0, i) for i in range(NWS)]
        accs = []
        act = None
        for c in range(TPV):
            for k, (kind, fc, i) in enumerate(fill):
                if k * TPV // len(fill) != c:
                    continue
                if kind == "gate":
                    act = ffn_gate(fc, i * QT, QT)
                elif kind == "up":
                    ffn_up(fc, act, i * QT, QT)
                else:
                    assert pv >= (NITEM - 1) * NC
                    r0, n = i * D // NWS, D // NWS
                    accs.append(acc_ref[zl, r0:r0 + n, 0:QT] + wo_proj(0, r0, n))
            do_pv(pv)
            if pv == (NITEM - 1) * NC - 1:
                finish(NITEM - 2)
            pv += 1
        acc = ffn_down(NHEAD * FC, F) + x_v[:, pl.ds(q0, BQ)].astype(f32)
        out_v[:, pl.ds(q0, QT)] = (jnp.concatenate(accs, axis=0) + acc[:, 0:QT]).astype(bf16)
        out_copy(b, 0).start()
        finish(NITEM - 1)
        acc = (acc[:, QT:BQ] + acc_ref[zl, :, QT:BQ]) + wo_proj(1)
        out_v[:, pl.ds(pl.multiple_of(q0 + QT, QT), QT)] = acc.astype(bf16)
        out_copy(b, 1).start()
        s_all[0, 0:16, 0:QT] = acc[0:16]
        return carry

    jax.lax.fori_loop(0, S // BQ, body, 0)
    for b in range(S // BQ):
        for t in range(NT):
            out_copy(b, t).wait()


@jax.jit
def pallas_parallel_sum__softmax_full_mha__glu_gated_swiglu__prompt_kernel(
    A_x: jax.Array,
    A_wqkv: jax.Array,
    A_wo: jax.Array,
    B_x: jax.Array,
    B_w1: jax.Array,
    B_w3: jax.Array,
    B_w2: jax.Array,
):
    del B_x
    xt = A_x.reshape(S, D).T
    hbm_spec = pl.BlockSpec(memory_space=pltpu.MemorySpace.HBM)
    out = pl.pallas_call(
        _kernel,
        out_shape=jax.ShapeDtypeStruct((D, S), bf16),
        in_specs=[hbm_spec] * 6,
        out_specs=hbm_spec,
        scratch_shapes=[
            pltpu.VMEM((D, S), bf16),
            pltpu.VMEM((D, 3 * D), bf16),
            pltpu.VMEM((D, D), bf16),
            pltpu.VMEM((D, F), bf16),
            pltpu.VMEM((D, F), bf16),
            pltpu.VMEM((D, F), bf16),
            pltpu.VMEM((S // 2, D), u32),
            pltpu.VMEM((BQ // 2, D), u32),
            pltpu.VMEM((3 * D // 2, D), u32),
            pltpu.VMEM((D // 2, H * HP), u32),
            pltpu.VMEM((D, TT), f32),
            pltpu.VMEM((256, TT), f32),
            pltpu.VMEM((G, S // 2, 128), u32),
            pltpu.VMEM((H, HP // 2, S), u32),
            pltpu.VMEM((1, QR + H * SVR, BQ), f32),
            pltpu.VMEM((H, HP // 2, S), u32),
            pltpu.VMEM((D, C, 128), f32),
            pltpu.VMEM((D, EX, 128), f32),
            pltpu.VMEM((H, HP // 2, BQ), u32),
            pltpu.VMEM((BQ // 2, F), u32),
            pltpu.VMEM((1, D, BQ), f32),
            pltpu.VMEM((D, S), bf16),
            pltpu.SMEM((2,), jnp.int32),
            pltpu.SemaphoreType.DMA((6,)),
            pltpu.VMEM((NBUF, S, W), f32),
        ],
        compiler_params=pltpu.CompilerParams(vmem_limit_bytes=120 * 1024 * 1024),
    )(xt, A_wqkv, A_wo, B_w1, B_w3, B_w2.T)
    return out.T.reshape(1, S, D)
```

```python
import math

import jax
import jax.numpy as jnp
import jax.experimental.pallas as pl
import jax.experimental.pallas.tpu as pltpu

S = 2048
D = 448
H = 16
DH = D // H
F = 1792
G = 4
HP = 32
QT = 128
W = 4 * QT
BQ = 256
NT = BQ // QT
NITEM = NT * G
C = 128
NC = S // C
EX = 64
NOFF = C + EX
NBUF = 6
TT = 128
FC = 128
NFFN = F // FC
NHEAD = NFFN - 2
X0 = 512
WA = 512
QR = H * HP
SVR = NOFF + 8
EPS = 1e-5
QSCALE = (DH ** -0.5) * math.log2(math.e)

L0 = 44
LAG = 3
HB = 1
TPV = 18
SPL = 4
QK_SPREAD = (1, 2, 2, 2, 2, 3, 3)
Q_AHEAD = 5
NWS = 7
GB = 8
KB_WEIGHTS = (2, 2, 2) + (3,) * 12

_NT_DIMS = (((1,), (1,)), ((), ()))
f32 = jnp.float32
bf16 = jnp.bfloat16
u32 = jnp.uint32


def _ex_lo(g):
    return 0 if g < G // 2 else C - EX


def _schedule():
    nq = NC - 1
    nqk = (NITEM - 1) * nq
    npv = NITEM * NC - TPV
    pos = []
    for p in range(npv):
        q = L0 + (p * (nqk - L0)) // (npv - 1)
        pos.append(max(q, min(nqk, (p // NC) * nq + LAG), pos[-1] if pos else 0))
    for it in range(NITEM):
        a, e = it * NC, min(npv, (it + 1) * NC)
        if a >= npv:
            break
        nxt = pos[e] if e < npv else nqk
        if e < npv and pos[e] == (it + 1) * nq + LAG:
            nxt = pos[e] - LAG
        for p in range(a, e):
            pos[p] = pos[a] + ((p - a) * (nxt - pos[a])) // max(1, e - a - 1)
    fine = []
    for it in range(NITEM):
        a, e = it * NC, min(npv, (it + 1) * NC)
        if a >= npv:
            break
        clamped = e < npv and pos[e] == (it + 1) * nq + LAG
        if e < npv and not clamped:
            span, den = pos[e] - pos[a], e - a
        else:
            span, den = pos[e - 1] - pos[a], max(1, e - a - 1)
        fine += [SPL * (pos[a] + nq) + ((p - a) * span * SPL) // den for p in range(a, e)]
    pos = [q + nq for q in pos]
    ntot = NITEM * nq
    slots = [None] * ntot
    for it in range(NITEM):
        end = min(pos[it * NC] - LAG, ntot) if it * NC < npv else ntot
        for i in range(HB):
            slots[end - HB + i] = (it, NC - HB + i)
    rest = iter([(it, c) for it in range(NITEM) for c in range(1, NC - HB)])
    slots = [s if s is not None else next(rest) for s in slots]
    seen = {}
    for k, (it, c) in enumerate(slots):
        assert c == seen.get(it, 0) + 1
        seen[it] = c
        if c == 1 and it >= NBUF:
            assert pos[(it - NBUF + 1) * NC - 1] <= k
        if c == NC - 1 and it * NC < npv:
            assert k < pos[it * NC]
    return slots, pos, fine


_SLOTS, _PV_POS, _FINE = _schedule()


def _pk(x):
    return pltpu.bitcast(x, u32)


def _up(x):
    return pltpu.bitcast(x, bf16)


def _kernel(x_hbm, wqkv_hbm, wo_hbm, w1_hbm, w3_hbm, w2_hbm, out_hbm,
            x_v, wqkv_v, wo_v, w1_v, w3_v, w2_v,
            xn_p, xc_p, wt_p, wot_p, kt32, kx32,
            k_p, qt_p, qs_ref, vt_p, kb_ref, kbx_ref,
            ot_p, h_p, acc_ref, out_v, z_ref, sems, s_all):
    def cols_copy(src, dst, lo, n, sem):
        return pltpu.make_async_copy(src.at[:, pl.ds(lo, n)], dst.at[:, pl.ds(lo, n)], sem)

    cp_x0 = cols_copy(x_hbm, x_v, 0, X0, sems.at[0])
    cp_wa = cols_copy(wqkv_hbm, wqkv_v, 0, WA, sems.at[1])
    cp_wb = cols_copy(wqkv_hbm, wqkv_v, WA, 3 * D - WA, sems.at[2])
    cp_x1 = cols_copy(x_hbm, x_v, X0, S - X0, sems.at[3])
    cp_wo = pltpu.make_async_copy(wo_hbm, wo_v, sems.at[3])
    cp_w1 = pltpu.make_async_copy(w1_hbm, w1_v, sems.at[4])
    cp_w3 = pltpu.make_async_copy(w3_hbm, w3_v, sems.at[4])
    cp_w2 = pltpu.make_async_copy(w2_hbm, w2_v, sems.at[4])
    cp_x0.start()
    cp_wa.start()
    cp_wb.start()
    cp_x1.start()
    z_ref[0] = 0
    z_ref[1] = 0
    s_all[0, 0:16, 0:QT] = jnp.zeros((16, QT), f32)

    false_row = []

    def store_xn(n, xnt):
        xn_p[n * TT // 2:(n + 1) * TT // 2, :] = _pk(xnt.T)

    def layernorm(n, pin=None):
        x = x_v[:, n * TT:(n + 1) * TT].astype(f32)
        if pin is not None:
            x = jnp.concatenate([jnp.where(false_row[0], pin, x[0:8]), x[8:]], axis=0)
        mu = jnp.mean(x, axis=0, keepdims=True)
        xc = x - mu
        var = jnp.mean(xc * xc, axis=0, keepdims=True)
        if not false_row:
            false_row.append(var < -1.0)
        return (xc * jax.lax.rsqrt(var + EPS)).astype(bf16)

    row4 = jax.lax.broadcasted_iota(jnp.int32, (HP - DH, TT), 0)
    z4 = jnp.zeros((HP - DH, TT), f32)
    one4 = jnp.where(row4 == 0, 1.0, 0.0).astype(f32)

    def qkv_proj(n, xnt, do_q=True, do_kv=True):
        cols = slice(n * TT, (n + 1) * TT)
        r0 = 0 if do_q else D
        r1 = 3 * D if do_kv else D
        qkv = jnp.dot(_up(wt_p[r0 // 2:r1 // 2, :]), xnt, preferred_element_type=f32)
        if do_q:
            for h in range(H):
                q = qkv[DH * h:DH * (h + 1)] * QSCALE
                qt_p[h, :, cols] = _pk(jnp.concatenate([q, z4], axis=0).astype(bf16))
        if do_kv:
            ko = D - r0
            vo = 2 * D - r0
            if n == 0:
                kt32[...] = qkv[ko:ko + D]
            else:
                if n == 1:
                    lane = jax.lax.broadcasted_iota(jnp.int32, (D // 2, TT), 1)
                    kx32[0:D // 2, :] = jnp.where(lane >= TT // 2, qkv[ko + D // 2:ko + D],
                                                  qkv[ko:ko + D // 2])
                for g in range(G):
                    parts = []
                    for j in range(4):
                        h = 4 * g + j
                        parts += [qkv[ko + DH * h:ko + DH * (h + 1)], z4]
                    k_p[g, n * TT // 2:(n + 1) * TT // 2, :] = _pk(
                        jnp.concatenate(parts, axis=0).astype(bf16).T)
            for h in range(H):
                v = qkv[vo + DH * h:vo + DH * (h + 1)]
                vt_p[h, :, cols] = _pk(jnp.concatenate([v, one4], axis=0).astype(bf16))
        return qkv[0:8], qkv[r1 - r0 - 8:r1 - r0]

    def kb_gen(lo, hi, pin):
        for r in range(lo, hi):
            src = kt32[r:r + 1, :] if r < D else kx32[r - D:r - D + 1, :]
            row8 = jnp.where(false_row[0], pin, jnp.broadcast_to(src, (8, TT)))
            kb = jnp.concatenate([row8] * (TT // 8), axis=0).astype(bf16).T
            if r < D:
                kb_ref[r] = kb.astype(f32)
            else:
                kbx_ref[r - D] = kb[0:EX].astype(f32)
                kbx_ref[r - D + D // 2] = kb[C - EX:C].astype(f32)

    ntile = S // TT
    n0 = X0 // TT
    cp_x0.wait()
    xnts = [layernorm(n) for n in range(n0)]
    cp_wa.wait()
    wt_p[0:WA // 2, :] = _pk(wqkv_v[:, 0:WA].T)
    for n in range(n0 - 1):
        qkv_proj(n, xnts[n], do_kv=False)
    for n in range(n0):
        store_xn(n, xnts[n])
    cp_wb.wait()
    cp_wo.start()
    cp_w1.start()
    cp_w3.start()
    cp_w2.start()
    wt_p[WA // 2:3 * D // 2, :] = _pk(wqkv_v[:, WA:3 * D].T)
    qkv_proj(n0 - 1, xnts[n0 - 1], do_kv=False)
    pins = []
    for n in range(ntile):
        if n == n0 - 1:
            cp_x1.wait()
            cp_wo.wait()
        if n < n0:
            xnt = xnts[n]
        else:
            xnt = layernorm(n, pins[n - 2][1])
            store_xn(n, xnt)
        pins.append(qkv_proj(n, xnt, do_q=(n >= n0)))
        if n >= 1:
            nrow, tot = D + D // 2, sum(KB_WEIGHTS)
            kb_gen(sum(KB_WEIGHTS[:n - 1]) * nrow // tot, sum(KB_WEIGHTS[:n]) * nrow // tot,
                   pins[n][0])
        if n == ntile - 2:
            wo32 = wo_v[...].astype(f32)
            z4w = jnp.zeros((HP - DH, D), f32)
            parts = []
            for h in range(H):
                parts += [wo32[DH * h:DH * (h + 1), :], z4w]
            wot_p[...] = _pk(jnp.concatenate(parts, axis=0).astype(bf16).T)
    cp_w1.wait()
    cp_w3.wait()
    cp_w2.wait()

    def out_copy(b, t):
        r0 = pl.multiple_of(b * BQ + t * QT, QT)
        return pltpu.make_async_copy(out_v.at[:, pl.ds(r0, QT)],
                                     out_hbm.at[:, pl.ds(r0, QT)], sems.at[5])

    def body(b, carry):
        q0 = pl.multiple_of(b * BQ, BQ)
        zs = z_ref[0]
        zl = z_ref[1]
        never = jax.lax.broadcasted_iota(jnp.int32, (16, QT), 1) < zs

        def stage_q(h):
            qs_ref[0, HP * h:HP * (h + 1), :] = _up(qt_p[h, :, pl.ds(q0, BQ)]).astype(f32)

        for h in reversed(range(H - Q_AHEAD, H)):
            stage_q(h)
        xc_p[...] = xn_p[pl.ds(pl.multiple_of(b * (BQ // 2), BQ // 2), BQ // 2), :]

        def vpu_scores():
            chain = s_all[0, 0:16, 0:QT]
            pending = []
            for t in reversed(range(NT)):
                cs = slice(t * QT, (t + 1) * QT)
                for h in reversed(range(H)):
                    qr = [qs_ref[0, HP * h + d:HP * h + d + 1, cs] for d in range(DH)]
                    vmax = None
                    for r in range(NOFF // 16):
                        src, rr = (kb_ref, r) if r < C // 16 else (kbx_ref, r - C // 16)
                        acc = None
                        for d in range(0, DH, 4):
                            if d % GB == 0:
                                nb = min(GB, DH - d)
                                kb = src[DH * h + d:DH * h + d + nb, rr * 16:(rr + 1) * 16, :]
                                kb = kb.reshape(nb * 16, QT)
                            p0, p1, p2, p3 = [
                                kb[(d % GB + i) * 16:(d % GB + i + 1) * 16] * qr[d + i]
                                for i in range(4)]
                            acc = jax.lax.select(never, chain, p0) if acc is None else acc + p0
                            acc = (acc + p1) + (p2 + p3)
                        chain = acc
                        vmax = acc if vmax is None else jnp.maximum(vmax, acc)
                        pending.append((QR + h * SVR + r * 16, cs, acc))
                    pending.append((QR + h * SVR + NOFF, cs, jnp.maximum(vmax[0:8], vmax[8:16])))
                    if t == NT - 1 and h >= Q_AHEAD:
                        stage_q(h - Q_AHEAD)
                    while len(pending) > 2:
                        row, cols, val = pending.pop(0)
                        qs_ref[zs, row:row + val.shape[0], cols] = val
            for row, cols, val in pending:
                qs_ref[zs, row:row + val.shape[0], cols] = val

        def q_weights(it):
            g, t = it // NT, it % NT
            cols = []
            for j in range(4):
                qj = _up(qt_p[4 * g + j, :, pl.ds(q0 + t * QT, QT)])
                parts = []
                if j > 0:
                    parts.append(jnp.zeros((HP * j, QT), bf16))
                parts.append(qj)
                if j < 3:
                    parts.append(jnp.zeros((HP * (3 - j), QT), bf16))
                cols.append(jnp.concatenate(parts, axis=0))
            return jnp.concatenate(cols, axis=1)

        qms, mruns, ms, outs = {}, {}, {}, {}

        def do_qk(k, cnt=1, part=None):
            it, c = _SLOTS[k]
            if c == 1:
                if it not in qms:
                    qms[it] = q_weights(it)
                lo = C + (EX if _ex_lo(it // NT) == 0 else 0)
                n = C - EX
            else:
                lo, n = c * C, cnt * C
            dst = c * C
            if part is not None:
                a0 = (n // 16 * part[0] // SPL) * 16
                a1 = (n // 16 * part[1] // SPL) * 16
                lo, dst, n = lo + a0, dst + a0, a1 - a0
            s = jnp.dot(_up(k_p[it // NT, lo // 2:(lo + n) // 2, :]), qms[it],
                        preferred_element_type=f32)
            s_all[it % NBUF, dst:dst + n, :] = s
            mc = jnp.max(s.reshape(n // 8, 8, W), axis=0)
            mruns[it] = mc if it not in mruns else jnp.maximum(mruns[it], mc)

        def do_qk_run(k0, k1):
            k = k0
            while k < k1:
                it, c = _SLOTS[k]
                cnt = 1
                while c > 1 and k + cnt < k1 and _SLOTS[k + cnt] == (it, c + cnt):
                    cnt += 1
                do_qk(k, cnt)
                k += cnt

        def do_pv(p):
            it, c = p // NC, p % NC
            g, t = it // NT, it % NT
            ts = slice(t * QT, (t + 1) * QT)
            if c == 0:
                vm = jnp.concatenate(
                    [qs_ref[0, QR + (4 * g + j) * SVR + NOFF:QR + (4 * g + j + 1) * SVR, ts]
                     for j in range(4)], axis=1)
                ms[it] = jnp.max(jnp.maximum(mruns[it], vm), axis=0, keepdims=True)
            oc = []
            for j in range(4):
                cs = slice(j * QT, (j + 1) * QT)
                r0 = QR + (4 * g + j) * SVR
                if c == 0:
                    s = qs_ref[0, r0:r0 + C, ts]
                elif c == 1:
                    parts = [qs_ref[0, r0 + C:r0 + NOFF, ts], s_all[it % NBUF, C:2 * C - EX, cs]]
                    s = jnp.concatenate(parts if _ex_lo(g) == 0 else parts[::-1], axis=0)
                else:
                    s = s_all[it % NBUF, c * C:(c + 1) * C, cs]
                pr = jnp.exp2(s - ms[it][:, cs]).astype(bf16)
                oc.append(jnp.dot(_up(vt_p[4 * g + j, :, c * C:(c + 1) * C]), pr,
                                  preferred_element_type=f32))
            outs[it] = oc if c == 0 else [a + e for a, e in zip(outs[it], oc)]

        def finish(it):
            g, t = it // NT, it % NT
            for j, o in enumerate(outs[it]):
                inv = 1.0 / o[DH:DH + 1, :]
                ot_p[4 * g + j, :, t * QT:(t + 1) * QT] = _pk((o * inv).astype(bf16))

        def ffn_gate(c, r0=0, n=BQ):
            xn = _up(xc_p[r0 // 2:(r0 + n) // 2, :])
            gate = jnp.dot(xn, w1_v[:, c * FC:(c + 1) * FC], preferred_element_type=f32)
            hg = 0.5 * gate
            return hg * jnp.tanh(hg) + hg

        def ffn_up(c, act, r0=0, n=BQ):
            xn = _up(xc_p[r0 // 2:(r0 + n) // 2, :])
            cols = slice(c * FC, (c + 1) * FC)
            up = jnp.dot(xn, w3_v[:, cols], preferred_element_type=f32)
            h_p[r0 // 2:(r0 + n) // 2, cols] = _pk((act * up).astype(bf16))

        def ffn_down(lo, hi):
            return jax.lax.dot_general(w2_v[:, lo:hi], _up(h_p[:, lo:hi]), _NT_DIMS,
                                       preferred_element_type=f32)

        def wo_proj(t, r0=0, n=D):
            ot = _up(ot_p[:, :, t * QT:(t + 1) * QT].reshape(H * HP // 2, QT))
            return jnp.dot(_up(wot_p[r0 // 2:(r0 + n) // 2, :]), ot, preferred_element_type=f32)

        vpu_scores()
        dn = None
        nq = 0
        for i in range(NHEAD // 2 + 1):
            if i < NHEAD // 2:
                for c in (2 * i, 2 * i + 1):
                    ffn_up(c, ffn_gate(c))
            do_qk_run(nq, nq + QK_SPREAD[i])
            nq += QK_SPREAD[i]
            if i > 0:
                part = ffn_down(2 * (i - 1) * FC, 2 * i * FC)
                dn = part if dn is None else dn + part
        acc_ref[zs] = dn
        do_qk_run(nq, _PV_POS[0])

        pv = 0
        for k in range(_PV_POS[0], len(_SLOTS) + 1):
            i = 0
            while True:
                while pv < len(_FINE) and _FINE[pv] <= k * SPL + i:
                    do_pv(pv)
                    if pv % NC == NC - 1:
                        finish(pv // NC)
                    pv += 1
                if k == len(_SLOTS) or i == SPL:
                    break
                j = i + 1
                while j < SPL and not (pv < len(_FINE) and _FINE[pv] <= k * SPL + j):
                    j += 1
                do_qk(k, part=(i, j))
                i = j
                if i == SPL:
                    break

        fill = [(kind, c, i) for c in range(NHEAD, NFFN) for i in range(NT)
                for kind in ("gate", "up")]
        fill += [("wo", 0, i) for i in range(NWS)]
        accs = []
        act = None
        for c in range(TPV):
            for k, (kind, fc, i) in enumerate(fill):
                if k * TPV // len(fill) != c:
                    continue
                if kind == "gate":
                    act = ffn_gate(fc, i * QT, QT)
                elif kind == "up":
                    ffn_up(fc, act, i * QT, QT)
                else:
                    assert pv >= (NITEM - 1) * NC
                    r0, n = i * D // NWS, D // NWS
                    accs.append(acc_ref[zl, r0:r0 + n, 0:QT] + wo_proj(0, r0, n))
            do_pv(pv)
            if pv == (NITEM - 1) * NC - 1:
                finish(NITEM - 2)
            pv += 1
        acc = ffn_down(NHEAD * FC, F) + x_v[:, pl.ds(q0, BQ)].astype(f32)
        out_v[:, pl.ds(q0, QT)] = (jnp.concatenate(accs, axis=0) + acc[:, 0:QT]).astype(bf16)
        out_copy(b, 0).start()
        finish(NITEM - 1)
        acc = (acc[:, QT:BQ] + acc_ref[zl, :, QT:BQ]) + wo_proj(1)
        out_v[:, pl.ds(pl.multiple_of(q0 + QT, QT), QT)] = acc.astype(bf16)
        out_copy(b, 1).start()
        s_all[0, 0:16, 0:QT] = acc[0:16]
        return carry

    jax.lax.fori_loop(0, S // BQ, body, 0)
    for b in range(S // BQ):
        for t in range(NT):
            out_copy(b, t).wait()


@jax.jit
def pallas_parallel_sum__softmax_full_mha__glu_gated_swiglu__prompt_kernel(
    A_x: jax.Array,
    A_wqkv: jax.Array,
    A_wo: jax.Array,
    B_x: jax.Array,
    B_w1: jax.Array,
    B_w3: jax.Array,
    B_w2: jax.Array,
):
    del B_x
    xt = A_x.reshape(S, D).T
    hbm_spec = pl.BlockSpec(memory_space=pltpu.MemorySpace.HBM)
    out = pl.pallas_call(
        _kernel,
        out_shape=jax.ShapeDtypeStruct((D, S), bf16),
        in_specs=[hbm_spec] * 6,
        out_specs=hbm_spec,
        scratch_shapes=[
            pltpu.VMEM((D, S), bf16),
            pltpu.VMEM((D, 3 * D), bf16),
            pltpu.VMEM((D, D), bf16),
            pltpu.VMEM((D, F), bf16),
            pltpu.VMEM((D, F), bf16),
            pltpu.VMEM((D, F), bf16),
            pltpu.VMEM((S // 2, D), u32),
            pltpu.VMEM((BQ // 2, D), u32),
            pltpu.VMEM((3 * D // 2, D), u32),
            pltpu.VMEM((D // 2, H * HP), u32),
            pltpu.VMEM((D, TT), f32),
            pltpu.VMEM((256, TT), f32),
            pltpu.VMEM((G, S // 2, 128), u32),
            pltpu.VMEM((H, HP // 2, S), u32),
            pltpu.VMEM((1, QR + H * SVR, BQ), f32),
            pltpu.VMEM((H, HP // 2, S), u32),
            pltpu.VMEM((D, C, 128), f32),
            pltpu.VMEM((D, EX, 128), f32),
            pltpu.VMEM((H, HP // 2, BQ), u32),
            pltpu.VMEM((BQ // 2, F), u32),
            pltpu.VMEM((1, D, BQ), f32),
            pltpu.VMEM((D, S), bf16),
            pltpu.SMEM((2,), jnp.int32),
            pltpu.SemaphoreType.DMA((6,)),
            pltpu.VMEM((NBUF, S, W), f32),
        ],
        compiler_params=pltpu.CompilerParams(vmem_limit_bytes=120 * 1024 * 1024),
    )(xt, A_wqkv, A_wo, B_w1, B_w3, B_w2.T)
    return out.T.reshape(1, S, D)
```

```python
import math

import jax
import jax.numpy as jnp
import jax.experimental.pallas as pl
import jax.experimental.pallas.tpu as pltpu

S = 2048
D = 448
H = 16
DH = D // H
F = 1792
G = 4
HP = 32
QT = 128
W = 4 * QT
BQ = 256
NT = BQ // QT
NITEM = NT * G
C = 128
NC = S // C
EX = 64
NOFF = C + EX
NBUF = 6
TT = 128
FC = 128
NFFN = F // FC
NHEAD = NFFN - 2
X0 = 512
WA = 512
QR = H * HP
SVR = NOFF + 8
EPS = 1e-5
QSCALE = (DH ** -0.5) * math.log2(math.e)

L0 = 44
LAG = 3
HB = 1
TPV = 18
SPL = 4
QK_SPREAD = (1, 2, 2, 2, 2, 3, 3)
Q_AHEAD = 5
NWS = 7
GB = 8
KB_WEIGHTS = (2, 2, 2) + (3,) * 12

_NT_DIMS = (((1,), (1,)), ((), ()))
f32 = jnp.float32
bf16 = jnp.bfloat16
u32 = jnp.uint32


def _ex_lo(g):
    return 0 if g < G // 2 else C - EX


def _schedule():
    nq = NC - 1
    nqk = (NITEM - 1) * nq
    npv = NITEM * NC - TPV
    pos = []
    for p in range(npv):
        q = L0 + (p * (nqk - L0)) // (npv - 1)
        pos.append(max(q, min(nqk, (p // NC) * nq + LAG), pos[-1] if pos else 0))
    for it in range(NITEM):
        a, e = it * NC, min(npv, (it + 1) * NC)
        if a >= npv:
            break
        nxt = pos[e] if e < npv else nqk
        if e < npv and pos[e] == (it + 1) * nq + LAG:
            nxt = pos[e] - LAG
        for p in range(a, e):
            pos[p] = pos[a] + ((p - a) * (nxt - pos[a])) // max(1, e - a - 1)
    fine = []
    for it in range(NITEM):
        a, e = it * NC, min(npv, (it + 1) * NC)
        if a >= npv:
            break
        clamped = e < npv and pos[e] == (it + 1) * nq + LAG
        if e < npv and not clamped:
            span, den = pos[e] - pos[a], e - a
        else:
            span, den = pos[e - 1] - pos[a], max(1, e - a - 1)
        fine += [SPL * (pos[a] + nq) + ((p - a) * span * SPL) // den for p in range(a, e)]
    pos = [q + nq for q in pos]
    ntot = NITEM * nq
    slots = [None] * ntot
    for it in range(NITEM):
        end = min(pos[it * NC] - LAG, ntot) if it * NC < npv else ntot
        for i in range(HB):
            slots[end - HB + i] = (it, NC - HB + i)
    rest = iter([(it, c) for it in range(NITEM) for c in range(1, NC - HB)])
    slots = [s if s is not None else next(rest) for s in slots]
    seen = {}
    for k, (it, c) in enumerate(slots):
        assert c == seen.get(it, 0) + 1
        seen[it] = c
        if c == 1 and it >= NBUF:
            assert pos[(it - NBUF + 1) * NC - 1] <= k
        if c == NC - 1 and it * NC < npv:
            assert k < pos[it * NC]
    return slots, pos, fine


_SLOTS, _PV_POS, _FINE = _schedule()


def _pk(x):
    return pltpu.bitcast(x, u32)


def _up(x):
    return pltpu.bitcast(x, bf16)


@jax.jit
def _mac(acc, kb, q, never):
    kb = kb.reshape(len(q) * 16, QT)
    for d in range(0, len(q), 4):
        p0, p1, p2, p3 = [kb[(d + i) * 16:(d + i + 1) * 16] * q[d + i] for i in range(4)]
        if d == 0 and never is not None:
            acc = jax.lax.select(never, acc, p0)
        else:
            acc = acc + p0
        acc = (acc + p1) + (p2 + p3)
    return acc


def _kernel(x_hbm, wqkv_hbm, wo_hbm, w1_hbm, w3_hbm, w2_hbm, out_hbm,
            x_v, wqkv_v, wo_v, w1_v, w3_v, w2_v,
            xn_p, xc_p, wt_p, wot_p, kt32, kx32,
            k_p, qt_p, qs_ref, vt_p, kb_ref, kbx_ref,
            ot_p, h_p, acc_ref, out_v, z_ref, sems, s_all):
    def cols_copy(src, dst, lo, n, sem):
        return pltpu.make_async_copy(src.at[:, pl.ds(lo, n)], dst.at[:, pl.ds(lo, n)], sem)

    cp_x0 = cols_copy(x_hbm, x_v, 0, X0, sems.at[0])
    cp_wa = cols_copy(wqkv_hbm, wqkv_v, 0, WA, sems.at[1])
    cp_wb = cols_copy(wqkv_hbm, wqkv_v, WA, 3 * D - WA, sems.at[2])
    cp_x1 = cols_copy(x_hbm, x_v, X0, S - X0, sems.at[3])
    cp_wo = pltpu.make_async_copy(wo_hbm, wo_v, sems.at[3])
    cp_w1 = pltpu.make_async_copy(w1_hbm, w1_v, sems.at[4])
    cp_w3 = pltpu.make_async_copy(w3_hbm, w3_v, sems.at[4])
    cp_w2 = pltpu.make_async_copy(w2_hbm, w2_v, sems.at[4])
    cp_x0.start()
    cp_wa.start()
    cp_wb.start()
    cp_x1.start()
    z_ref[0] = 0
    z_ref[1] = 0
    s_all[0, 0:16, 0:QT] = jnp.zeros((16, QT), f32)

    false_row = []

    def store_xn(n, xnt):
        xn_p[n * TT // 2:(n + 1) * TT // 2, :] = _pk(xnt.T)

    def layernorm(n, pin=None):
        x = x_v[:, n * TT:(n + 1) * TT].astype(f32)
        if pin is not None:
            x = jnp.concatenate([jnp.where(false_row[0], pin, x[0:8]), x[8:]], axis=0)
        mu = jnp.mean(x, axis=0, keepdims=True)
        xc = x - mu
        var = jnp.mean(xc * xc, axis=0, keepdims=True)
        if not false_row:
            false_row.append(var < -1.0)
        return (xc * jax.lax.rsqrt(var + EPS)).astype(bf16)

    row4 = jax.lax.broadcasted_iota(jnp.int32, (HP - DH, TT), 0)
    z4 = jnp.zeros((HP - DH, TT), f32)
    one4 = jnp.where(row4 == 0, 1.0, 0.0).astype(f32)

    def qkv_proj(n, xnt, do_q=True, do_kv=True):
        cols = slice(n * TT, (n + 1) * TT)
        r0 = 0 if do_q else D
        r1 = 3 * D if do_kv else D
        qkv = jnp.dot(_up(wt_p[r0 // 2:r1 // 2, :]), xnt, preferred_element_type=f32)
        if do_q:
            for h in range(H):
                q = qkv[DH * h:DH * (h + 1)] * QSCALE
                qt_p[h, :, cols] = _pk(jnp.concatenate([q, z4], axis=0).astype(bf16))
        if do_kv:
            ko = D - r0
            vo = 2 * D - r0
            if n == 0:
                kt32[...] = qkv[ko:ko + D]
            else:
                if n == 1:
                    lane = jax.lax.broadcasted_iota(jnp.int32, (D // 2, TT), 1)
                    kx32[0:D // 2, :] = jnp.where(lane >= TT // 2, qkv[ko + D // 2:ko + D],
                                                  qkv[ko:ko + D // 2])
                for g in range(G):
                    parts = []
                    for j in range(4):
                        h = 4 * g + j
                        parts += [qkv[ko + DH * h:ko + DH * (h + 1)], z4]
                    k_p[g, n * TT // 2:(n + 1) * TT // 2, :] = _pk(
                        jnp.concatenate(parts, axis=0).astype(bf16).T)
            for h in range(H):
                v = qkv[vo + DH * h:vo + DH * (h + 1)]
                vt_p[h, :, cols] = _pk(jnp.concatenate([v, one4], axis=0).astype(bf16))
        return qkv[0:8], qkv[r1 - r0 - 8:r1 - r0]

    def kb_gen(lo, hi, pin):
        for r in range(lo, hi):
            src = kt32[r:r + 1, :] if r < D else kx32[r - D:r - D + 1, :]
            row8 = jnp.where(false_row[0], pin, jnp.broadcast_to(src, (8, TT)))
            kb = jnp.concatenate([row8] * (TT // 8), axis=0).astype(bf16).T
            if r < D:
                kb_ref[r] = kb.astype(f32)
            else:
                kbx_ref[r - D] = kb[0:EX].astype(f32)
                kbx_ref[r - D + D // 2] = kb[C - EX:C].astype(f32)

    ntile = S // TT
    n0 = X0 // TT
    cp_x0.wait()
    xnts = [layernorm(n) for n in range(n0)]
    cp_wa.wait()
    wt_p[0:WA // 2, :] = _pk(wqkv_v[:, 0:WA].T)
    for n in range(n0 - 1):
        qkv_proj(n, xnts[n], do_kv=False)
    for n in range(n0):
        store_xn(n, xnts[n])
    cp_wb.wait()
    cp_wo.start()
    cp_w1.start()
    cp_w3.start()
    cp_w2.start()
    wt_p[WA // 2:3 * D // 2, :] = _pk(wqkv_v[:, WA:3 * D].T)
    qkv_proj(n0 - 1, xnts[n0 - 1], do_kv=False)
    pins = []
    for n in range(ntile):
        if n == n0 - 1:
            cp_x1.wait()
            cp_wo.wait()
        if n < n0:
            xnt = xnts[n]
        else:
            xnt = layernorm(n, pins[n - 2][1])
            store_xn(n, xnt)
        pins.append(qkv_proj(n, xnt, do_q=(n >= n0)))
        if n >= 1:
            nrow, tot = D + D // 2, sum(KB_WEIGHTS)
            kb_gen(sum(KB_WEIGHTS[:n - 1]) * nrow // tot, sum(KB_WEIGHTS[:n]) * nrow // tot,
                   pins[n][0])
        if n == ntile - 2:
            wo32 = wo_v[...].astype(f32)
            z4w = jnp.zeros((HP - DH, D), f32)
            parts = []
            for h in range(H):
                parts += [wo32[DH * h:DH * (h + 1), :], z4w]
            wot_p[...] = _pk(jnp.concatenate(parts, axis=0).astype(bf16).T)
    cp_w1.wait()
    cp_w3.wait()
    cp_w2.wait()

    def out_copy(b, t):
        r0 = pl.multiple_of(b * BQ + t * QT, QT)
        return pltpu.make_async_copy(out_v.at[:, pl.ds(r0, QT)],
                                     out_hbm.at[:, pl.ds(r0, QT)], sems.at[5])

    def body(b, carry):
        q0 = pl.multiple_of(b * BQ, BQ)
        zs = z_ref[0]
        zl = z_ref[1]
        never = jax.lax.broadcasted_iota(jnp.int32, (16, QT), 1) < zs

        def stage_q(h):
            qs_ref[0, HP * h:HP * (h + 1), :] = _up(qt_p[h, :, pl.ds(q0, BQ)]).astype(f32)

        for h in reversed(range(H - Q_AHEAD, H)):
            stage_q(h)
        xc_p[...] = xn_p[pl.ds(pl.multiple_of(b * (BQ // 2), BQ // 2), BQ // 2), :]

        def vpu_scores():
            chain = s_all[0, 0:16, 0:QT]
            pending = []
            for t in reversed(range(NT)):
                cs = slice(t * QT, (t + 1) * QT)
                for h in reversed(range(H)):
                    qr = [qs_ref[0, HP * h + d:HP * h + d + 1, cs] for d in range(DH)]
                    vmax = None
                    for r in range(NOFF // 16):
                        src, rr = (kb_ref, r) if r < C // 16 else (kbx_ref, r - C // 16)
                        acc = chain
                        for d in range(0, DH, GB):
                            nb = min(GB, DH - d)
                            kb = src[DH * h + d:DH * h + d + nb, rr * 16:(rr + 1) * 16, :]
                            acc = _mac(acc, kb, qr[d:d + nb], never if d == 0 else None)
                        chain = acc
                        vmax = acc if vmax is None else jnp.maximum(vmax, acc)
                        pending.append((QR + h * SVR + r * 16, cs, acc))
                    pending.append((QR + h * SVR + NOFF, cs, jnp.maximum(vmax[0:8], vmax[8:16])))
                    if t == NT - 1 and h >= Q_AHEAD:
                        stage_q(h - Q_AHEAD)
                    while len(pending) > 2:
                        row, cols, val = pending.pop(0)
                        qs_ref[zs, row:row + val.shape[0], cols] = val
            for row, cols, val in pending:
                qs_ref[zs, row:row + val.shape[0], cols] = val

        def q_weights(it):
            g, t = it // NT, it % NT
            cols = []
            for j in range(4):
                qj = _up(qt_p[4 * g + j, :, pl.ds(q0 + t * QT, QT)])
                parts = []
                if j > 0:
                    parts.append(jnp.zeros((HP * j, QT), bf16))
                parts.append(qj)
                if j < 3:
                    parts.append(jnp.zeros((HP * (3 - j), QT), bf16))
                cols.append(jnp.concatenate(parts, axis=0))
            return jnp.concatenate(cols, axis=1)

        qms, mruns, ms, outs = {}, {}, {}, {}

        def do_qk(k, cnt=1, part=None):
            it, c = _SLOTS[k]
            if c == 1:
                if it not in qms:
                    qms[it] = q_weights(it)
                lo = C + (EX if _ex_lo(it // NT) == 0 else 0)
                n = C - EX
            else:
                lo, n = c * C, cnt * C
            dst = c * C
            if part is not None:
                a0 = (n // 16 * part[0] // SPL) * 16
                a1 = (n // 16 * part[1] // SPL) * 16
                lo, dst, n = lo + a0, dst + a0, a1 - a0
            s = jnp.dot(_up(k_p[it // NT, lo // 2:(lo + n) // 2, :]), qms[it],
                        preferred_element_type=f32)
            s_all[it % NBUF, dst:dst + n, :] = s
            mc = jnp.max(s.reshape(n // 8, 8, W), axis=0)
            mruns[it] = mc if it not in mruns else jnp.maximum(mruns[it], mc)

        def do_qk_run(k0, k1):
            k = k0
            while k < k1:
                it, c = _SLOTS[k]
                cnt = 1
                while c > 1 and k + cnt < k1 and _SLOTS[k + cnt] == (it, c + cnt):
                    cnt += 1
                do_qk(k, cnt)
                k += cnt

        def do_pv(p):
            it, c = p // NC, p % NC
            g, t = it // NT, it % NT
            ts = slice(t * QT, (t + 1) * QT)
            if c == 0:
                vm = jnp.concatenate(
                    [qs_ref[0, QR + (4 * g + j) * SVR + NOFF:QR + (4 * g + j + 1) * SVR, ts]
                     for j in range(4)], axis=1)
                ms[it] = jnp.max(jnp.maximum(mruns[it], vm), axis=0, keepdims=True)
            oc = []
            for j in range(4):
                cs = slice(j * QT, (j + 1) * QT)
                r0 = QR + (4 * g + j) * SVR
                if c == 0:
                    s = qs_ref[0, r0:r0 + C, ts]
                elif c == 1:
                    parts = [qs_ref[0, r0 + C:r0 + NOFF, ts], s_all[it % NBUF, C:2 * C - EX, cs]]
                    s = jnp.concatenate(parts if _ex_lo(g) == 0 else parts[::-1], axis=0)
                else:
                    s = s_all[it % NBUF, c * C:(c + 1) * C, cs]
                pr = jnp.exp2(s - ms[it][:, cs]).astype(bf16)
                oc.append(jnp.dot(_up(vt_p[4 * g + j, :, c * C:(c + 1) * C]), pr,
                                  preferred_element_type=f32))
            outs[it] = oc if c == 0 else [a + e for a, e in zip(outs[it], oc)]

        def finish(it):
            g, t = it // NT, it % NT
            for j, o in enumerate(outs[it]):
                inv = 1.0 / o[DH:DH + 1, :]
                ot_p[4 * g + j, :, t * QT:(t + 1) * QT] = _pk((o * inv).astype(bf16))

        def ffn_gate(c, r0=0, n=BQ):
            xn = _up(xc_p[r0 // 2:(r0 + n) // 2, :])
            gate = jnp.dot(xn, w1_v[:, c * FC:(c + 1) * FC], preferred_element_type=f32)
            hg = 0.5 * gate
            return hg * jnp.tanh(hg) + hg

        def ffn_up(c, act, r0=0, n=BQ):
            xn = _up(xc_p[r0 // 2:(r0 + n) // 2, :])
            cols = slice(c * FC, (c + 1) * FC)
            up = jnp.dot(xn, w3_v[:, cols], preferred_element_type=f32)
            h_p[r0 // 2:(r0 + n) // 2, cols] = _pk((act * up).astype(bf16))

        def ffn_down(lo, hi):
            return jax.lax.dot_general(w2_v[:, lo:hi], _up(h_p[:, lo:hi]), _NT_DIMS,
                                       preferred_element_type=f32)

        def wo_proj(t, r0=0, n=D):
            ot = _up(ot_p[:, :, t * QT:(t + 1) * QT].reshape(H * HP // 2, QT))
            return jnp.dot(_up(wot_p[r0 // 2:(r0 + n) // 2, :]), ot, preferred_element_type=f32)

        vpu_scores()
        dn = None
        nq = 0
        for i in range(NHEAD // 2 + 1):
            if i < NHEAD // 2:
                for c in (2 * i, 2 * i + 1):
                    ffn_up(c, ffn_gate(c))
            do_qk_run(nq, nq + QK_SPREAD[i])
            nq += QK_SPREAD[i]
            if i > 0:
                part = ffn_down(2 * (i - 1) * FC, 2 * i * FC)
                dn = part if dn is None else dn + part
        acc_ref[zs] = dn
        do_qk_run(nq, _PV_POS[0])

        pv = 0
        for k in range(_PV_POS[0], len(_SLOTS) + 1):
            i = 0
            while True:
                while pv < len(_FINE) and _FINE[pv] <= k * SPL + i:
                    do_pv(pv)
                    if pv % NC == NC - 1:
                        finish(pv // NC)
                    pv += 1
                if k == len(_SLOTS) or i == SPL:
                    break
                j = i + 1
                while j < SPL and not (pv < len(_FINE) and _FINE[pv] <= k * SPL + j):
                    j += 1
                do_qk(k, part=(i, j))
                i = j
                if i == SPL:
                    break

        fill = [(kind, c, i) for c in range(NHEAD, NFFN) for i in range(NT)
                for kind in ("gate", "up")]
        fill += [("wo", 0, i) for i in range(NWS)]
        accs = []
        act = None
        for c in range(TPV):
            for k, (kind, fc, i) in enumerate(fill):
                if k * TPV // len(fill) != c:
                    continue
                if kind == "gate":
                    act = ffn_gate(fc, i * QT, QT)
                elif kind == "up":
                    ffn_up(fc, act, i * QT, QT)
                else:
                    assert pv >= (NITEM - 1) * NC
                    r0, n = i * D // NWS, D // NWS
                    accs.append(acc_ref[zl, r0:r0 + n, 0:QT] + wo_proj(0, r0, n))
            do_pv(pv)
            if pv == (NITEM - 1) * NC - 1:
                finish(NITEM - 2)
            pv += 1
        acc = ffn_down(NHEAD * FC, F) + x_v[:, pl.ds(q0, BQ)].astype(f32)
        out_v[:, pl.ds(q0, QT)] = (jnp.concatenate(accs, axis=0) + acc[:, 0:QT]).astype(bf16)
        out_copy(b, 0).start()
        finish(NITEM - 1)
        acc = (acc[:, QT:BQ] + acc_ref[zl, :, QT:BQ]) + wo_proj(1)
        out_v[:, pl.ds(pl.multiple_of(q0 + QT, QT), QT)] = acc.astype(bf16)
        out_copy(b, 1).start()
        s_all[0, 0:16, 0:QT] = acc[0:16]
        return carry

    jax.lax.fori_loop(0, S // BQ, body, 0)
    for b in range(S // BQ):
        for t in range(NT):
            out_copy(b, t).wait()


@jax.jit
def pallas_parallel_sum__softmax_full_mha__glu_gated_swiglu__prompt_kernel(
    A_x: jax.Array,
    A_wqkv: jax.Array,
    A_wo: jax.Array,
    B_x: jax.Array,
    B_w1: jax.Array,
    B_w3: jax.Array,
    B_w2: jax.Array,
):
    del B_x
    xt = A_x.reshape(S, D).T
    hbm_spec = pl.BlockSpec(memory_space=pltpu.MemorySpace.HBM)
    out = pl.pallas_call(
        _kernel,
        out_shape=jax.ShapeDtypeStruct((D, S), bf16),
        in_specs=[hbm_spec] * 6,
        out_specs=hbm_spec,
        scratch_shapes=[
            pltpu.VMEM((D, S), bf16),
            pltpu.VMEM((D, 3 * D), bf16),
            pltpu.VMEM((D, D), bf16),
            pltpu.VMEM((D, F), bf16),
            pltpu.VMEM((D, F), bf16),
            pltpu.VMEM((D, F), bf16),
            pltpu.VMEM((S // 2, D), u32),
            pltpu.VMEM((BQ // 2, D), u32),
            pltpu.VMEM((3 * D // 2, D), u32),
            pltpu.VMEM((D // 2, H * HP), u32),
            pltpu.VMEM((D, TT), f32),
            pltpu.VMEM((256, TT), f32),
            pltpu.VMEM((G, S // 2, 128), u32),
            pltpu.VMEM((H, HP // 2, S), u32),
            pltpu.VMEM((1, QR + H * SVR, BQ), f32),
            pltpu.VMEM((H, HP // 2, S), u32),
            pltpu.VMEM((D, C, 128), f32),
            pltpu.VMEM((D, EX, 128), f32),
            pltpu.VMEM((H, HP // 2, BQ), u32),
            pltpu.VMEM((BQ // 2, F), u32),
            pltpu.VMEM((1, D, BQ), f32),
            pltpu.VMEM((D, S), bf16),
            pltpu.SMEM((2,), jnp.int32),
            pltpu.SemaphoreType.DMA((6,)),
            pltpu.VMEM((NBUF, S, W), f32),
        ],
        compiler_params=pltpu.CompilerParams(vmem_limit_bytes=120 * 1024 * 1024),
    )(xt, A_wqkv, A_wo, B_w1, B_w3, B_w2.T)
    return out.T.reshape(1, S, D)
```

```python
import math

import jax
import jax.numpy as jnp
import jax.experimental.pallas as pl
import jax.experimental.pallas.tpu as pltpu

S = 2048
D = 448
H = 16
DH = D // H
F = 1792
G = 4
HP = 32
QT = 128
W = 4 * QT
BQ = 256
NT = BQ // QT
NITEM = NT * G
C = 128
NC = S // C
EX = 64
NOFF = C + EX
NBUF = 5
TT = 128
FC = 128
NFFN = F // FC
NHEAD = NFFN - 2
X0 = 512
WA = 512
QR = H * HP
SVR = NOFF + 8
EPS = 1e-5
QSCALE = (DH ** -0.5) * math.log2(math.e)

L0 = 44
LAG = 3
HB = 1
TPV = 18
SPL = 4
QK_SPREAD = (2, 2, 2, 2, 2, 3, 3)
Q_AHEAD = 5
NWS = 7
KB_WEIGHTS = (2, 2, 2) + (3,) * 12

_NT_DIMS = (((1,), (1,)), ((), ()))
f32 = jnp.float32
bf16 = jnp.bfloat16
u32 = jnp.uint32


def _ex_lo(g):
    return 0 if g < G // 2 else C - EX


def _schedule():
    nq = NC - 1
    nqk = (NITEM - 1) * nq
    npv = NITEM * NC - TPV
    pos = []
    for p in range(npv):
        q = L0 + (p * (nqk - L0)) // (npv - 1)
        pos.append(max(q, min(nqk, (p // NC) * nq + LAG), pos[-1] if pos else 0))
    for it in range(NITEM):
        a, e = it * NC, min(npv, (it + 1) * NC)
        if a >= npv:
            break
        nxt = pos[e] if e < npv else nqk
        if e < npv and pos[e] == (it + 1) * nq + LAG:
            nxt = pos[e] - LAG
        for p in range(a, e):
            pos[p] = pos[a] + ((p - a) * (nxt - pos[a])) // max(1, e - a - 1)
    fine = []
    for it in range(NITEM):
        a, e = it * NC, min(npv, (it + 1) * NC)
        if a >= npv:
            break
        clamped = e < npv and pos[e] == (it + 1) * nq + LAG
        if e < npv and not clamped:
            span, den = pos[e] - pos[a], e - a
        else:
            span, den = pos[e - 1] - pos[a], max(1, e - a - 1)
        fine += [SPL * (pos[a] + nq) + ((p - a) * span * SPL) // den for p in range(a, e)]
    pos = [q + nq for q in pos]
    ntot = NITEM * nq
    slots = [None] * ntot
    for it in range(NITEM):
        end = min(pos[it * NC] - LAG, ntot) if it * NC < npv else ntot
        for i in range(HB):
            slots[end - HB + i] = (it, NC - HB + i)
    rest = iter([(it, c) for it in range(NITEM) for c in range(1, NC - HB)])
    slots = [s if s is not None else next(rest) for s in slots]
    seen = {}
    for k, (it, c) in enumerate(slots):
        assert c == seen.get(it, 0) + 1
        seen[it] = c
        if c == 1 and it >= NBUF:
            assert pos[(it - NBUF + 1) * NC - 1] <= k
        if c == NC - 1 and it * NC < npv:
            assert k < pos[it * NC]
    return slots, pos, fine


_SLOTS, _PV_POS, _FINE = _schedule()


def _pk(x):
    return pltpu.bitcast(x, u32)


def _up(x):
    return pltpu.bitcast(x, bf16)


@jax.jit
def _scores16(kb, q, prev, never):
    kb = kb.reshape(DH * 16, QT)
    acc = None
    for d in range(0, DH, 4):
        p0, p1, p2, p3 = [kb[(d + i) * 16:(d + i + 1) * 16] * q[d + i] for i in range(4)]
        acc = jax.lax.select(never, prev, p0) if acc is None else acc + p0
        acc = (acc + p1) + (p2 + p3)
    return acc


def _kernel(x_hbm, wqkv_hbm, wo_hbm, w1_hbm, w3_hbm, w2_hbm, out_hbm,
            x_v, wqkv_v, wo_v, w1_v, w3_v, w2_v,
            xn_p, xc_p, wt_p, wot_p, kt32, kx32,
            k_p, qt_p, qs_ref, vt_p, kb_ref, kbx_ref,
            ot_p, h_p, acc_ref, out_v, z_ref, sems, s_all):
    def cols_copy(src, dst, lo, n, sem):
        return pltpu.make_async_copy(src.at[:, pl.ds(lo, n)], dst.at[:, pl.ds(lo, n)], sem)

    cp_x0 = cols_copy(x_hbm, x_v, 0, X0, sems.at[0])
    cp_wa = cols_copy(wqkv_hbm, wqkv_v, 0, WA, sems.at[1])
    cp_wb = cols_copy(wqkv_hbm, wqkv_v, WA, 3 * D - WA, sems.at[2])
    cp_x1 = cols_copy(x_hbm, x_v, X0, S - X0, sems.at[3])
    cp_wo = pltpu.make_async_copy(wo_hbm, wo_v, sems.at[3])
    cp_w1 = pltpu.make_async_copy(w1_hbm, w1_v, sems.at[4])
    cp_w3 = pltpu.make_async_copy(w3_hbm, w3_v, sems.at[4])
    cp_w2 = pltpu.make_async_copy(w2_hbm, w2_v, sems.at[4])
    cp_x0.start()
    cp_wa.start()
    cp_wb.start()
    cp_x1.start()
    z_ref[0] = 0
    z_ref[1] = 0
    s_all[0, 0:16, 0:QT] = jnp.zeros((16, QT), f32)

    false_row = []

    def store_xn(n, xnt):
        xn_p[n * TT // 2:(n + 1) * TT // 2, :] = _pk(xnt.T)

    def layernorm(n, pin=None):
        x = x_v[:, n * TT:(n + 1) * TT].astype(f32)
        if pin is not None:
            x = jnp.concatenate([jnp.where(false_row[0], pin, x[0:8]), x[8:]], axis=0)
        mu = jnp.mean(x, axis=0, keepdims=True)
        xc = x - mu
        var = jnp.mean(xc * xc, axis=0, keepdims=True)
        if not false_row:
            false_row.append(var < -1.0)
        return (xc * jax.lax.rsqrt(var + EPS)).astype(bf16)

    row4 = jax.lax.broadcasted_iota(jnp.int32, (HP - DH, TT), 0)
    z4 = jnp.zeros((HP - DH, TT), f32)
    one4 = jnp.where(row4 == 0, 1.0, 0.0).astype(f32)

    def qkv_proj(n, xnt, do_q=True, do_kv=True):
        cols = slice(n * TT, (n + 1) * TT)
        r0 = 0 if do_q else D
        r1 = 3 * D if do_kv else D
        qkv = jnp.dot(_up(wt_p[r0 // 2:r1 // 2, :]), xnt, preferred_element_type=f32)
        if do_q:
            for h in range(H):
                q = qkv[DH * h:DH * (h + 1)] * QSCALE
                qt_p[h, :, cols] = _pk(jnp.concatenate([q, z4], axis=0).astype(bf16))
        if do_kv:
            ko = D - r0
            vo = 2 * D - r0
            if n == 0:
                kt32[...] = qkv[ko:ko + D]
            else:
                if n == 1:
                    lane = jax.lax.broadcasted_iota(jnp.int32, (D // 2, TT), 1)
                    kx32[0:D // 2, :] = jnp.where(lane >= TT // 2, qkv[ko + D // 2:ko + D],
                                                  qkv[ko:ko + D // 2])
                for g in range(G):
                    parts = []
                    for j in range(4):
                        h = 4 * g + j
                        parts += [qkv[ko + DH * h:ko + DH * (h + 1)], z4]
                    k_p[g, n * TT // 2:(n + 1) * TT // 2, :] = _pk(
                        jnp.concatenate(parts, axis=0).astype(bf16).T)
            for h in range(H):
                v = qkv[vo + DH * h:vo + DH * (h + 1)]
                vt_p[h, :, cols] = _pk(jnp.concatenate([v, one4], axis=0).astype(bf16))
        return qkv[0:8], qkv[r1 - r0 - 8:r1 - r0]

    def kb_gen(lo, hi, pin):
        for r in range(lo, hi):
            src = kt32[r:r + 1, :] if r < D else kx32[r - D:r - D + 1, :]
            row8 = jnp.where(false_row[0], pin, jnp.broadcast_to(src, (8, TT)))
            kb = jnp.concatenate([row8] * (TT // 8), axis=0).astype(bf16).T
            if r < D:
                kb_ref[r] = kb.astype(f32)
            else:
                kbx_ref[r - D] = kb[0:EX].astype(f32)
                kbx_ref[r - D + D // 2] = kb[C - EX:C].astype(f32)

    ntile = S // TT
    n0 = X0 // TT
    cp_x0.wait()
    xnts = [layernorm(n) for n in range(n0)]
    cp_wa.wait()
    wt_p[0:WA // 2, :] = _pk(wqkv_v[:, 0:WA].T)
    for n in range(n0 - 1):
        qkv_proj(n, xnts[n], do_kv=False)
    for n in range(n0):
        store_xn(n, xnts[n])
    cp_wb.wait()
    cp_wo.start()
    cp_w1.start()
    cp_w3.start()
    cp_w2.start()
    wt_p[WA // 2:3 * D // 2, :] = _pk(wqkv_v[:, WA:3 * D].T)
    qkv_proj(n0 - 1, xnts[n0 - 1], do_kv=False)
    pins = []
    for n in range(ntile):
        if n == n0 - 1:
            cp_x1.wait()
            cp_wo.wait()
        if n < n0:
            xnt = xnts[n]
        else:
            xnt = layernorm(n, pins[n - 2][1])
            store_xn(n, xnt)
        pins.append(qkv_proj(n, xnt, do_q=(n >= n0)))
        if n >= 1:
            nrow, tot = D + D // 2, sum(KB_WEIGHTS)
            kb_gen(sum(KB_WEIGHTS[:n - 1]) * nrow // tot, sum(KB_WEIGHTS[:n]) * nrow // tot,
                   pins[n][0])
        if n == ntile - 2:
            wo32 = wo_v[...].astype(f32)
            z4w = jnp.zeros((HP - DH, D), f32)
            parts = []
            for h in range(H):
                parts += [wo32[DH * h:DH * (h + 1), :], z4w]
            wot_p[...] = _pk(jnp.concatenate(parts, axis=0).astype(bf16).T)
    cp_w1.wait()
    cp_w3.wait()
    cp_w2.wait()

    def out_copy(b, t):
        r0 = pl.multiple_of(b * BQ + t * QT, QT)
        return pltpu.make_async_copy(out_v.at[:, pl.ds(r0, QT)],
                                     out_hbm.at[:, pl.ds(r0, QT)], sems.at[5])

    def body(b, carry):
        q0 = pl.multiple_of(b * BQ, BQ)
        zs = z_ref[0]
        zl = z_ref[1]
        never = jax.lax.broadcasted_iota(jnp.int32, (16, QT), 1) < zs

        def stage_q(h):
            qs_ref[0, HP * h:HP * (h + 1), :] = _up(qt_p[h, :, pl.ds(q0, BQ)]).astype(f32)

        for h in reversed(range(H - Q_AHEAD, H)):
            stage_q(h)
        xc_p[...] = xn_p[pl.ds(pl.multiple_of(b * (BQ // 2), BQ // 2), BQ // 2), :]

        def vpu_scores():
            chain = s_all[0, 0:16, 0:QT]
            pending = []
            for t in reversed(range(NT)):
                cs = slice(t * QT, (t + 1) * QT)
                for h in reversed(range(H)):
                    qr = [qs_ref[0, HP * h + d:HP * h + d + 1, cs] for d in range(DH)]
                    vmax = None
                    for r in range(NOFF // 16):
                        src, rr = (kb_ref, r) if r < C // 16 else (kbx_ref, r - C // 16)
                        kb = src[DH * h:DH * (h + 1), rr * 16:(rr + 1) * 16, :]
                        acc = _scores16(kb, qr, chain, never)
                        chain = acc
                        vmax = acc if vmax is None else jnp.maximum(vmax, acc)
                        pending.append((QR + h * SVR + r * 16, cs, acc))
                    pending.append((QR + h * SVR + NOFF, cs, jnp.maximum(vmax[0:8], vmax[8:16])))
                    if t == NT - 1 and h >= Q_AHEAD:
                        stage_q(h - Q_AHEAD)
                    while len(pending) > 2:
                        row, cols, val = pending.pop(0)
                        qs_ref[zs, row:row + val.shape[0], cols] = val
            for row, cols, val in pending:
                qs_ref[zs, row:row + val.shape[0], cols] = val

        def q_weights(it):
            g, t = it // NT, it % NT
            cols = []
            for j in range(4):
                qj = _up(qt_p[4 * g + j, :, pl.ds(q0 + t * QT, QT)])
                parts = []
                if j > 0:
                    parts.append(jnp.zeros((HP * j, QT), bf16))
                parts.append(qj)
                if j < 3:
                    parts.append(jnp.zeros((HP * (3 - j), QT), bf16))
                cols.append(jnp.concatenate(parts, axis=0))
            return jnp.concatenate(cols, axis=1)

        qms, mruns, ms, outs = {}, {}, {}, {}

        def do_qk(k, cnt=1, part=None):
            it, c = _SLOTS[k]
            if c == 1:
                if it not in qms:
                    qms[it] = q_weights(it)
                lo = C + (EX if _ex_lo(it // NT) == 0 else 0)
                n = C - EX
            else:
                lo, n = c * C, cnt * C
            dst = c * C
            if part is not None:
                a0 = (n // 16 * part[0] // SPL) * 16
                a1 = (n // 16 * part[1] // SPL) * 16
                lo, dst, n = lo + a0, dst + a0, a1 - a0
            s = jnp.dot(_up(k_p[it // NT, lo // 2:(lo + n) // 2, :]), qms[it],
                        preferred_element_type=f32)
            s_all[it % NBUF, dst:dst + n, :] = s
            mc = jnp.max(s.reshape(n // 8, 8, W), axis=0)
            mruns[it] = mc if it not in mruns else jnp.maximum(mruns[it], mc)

        def do_qk_run(k0, k1):
            k = k0
            while k < k1:
                it, c = _SLOTS[k]
                cnt = 1
                while c > 1 and k + cnt < k1 and _SLOTS[k + cnt] == (it, c + cnt):
                    cnt += 1
                do_qk(k, cnt)
                k += cnt

        def do_pv(p):
            it, c = p // NC, p % NC
            g, t = it // NT, it % NT
            ts = slice(t * QT, (t + 1) * QT)
            if c == 0:
                vm = jnp.concatenate(
                    [qs_ref[0, QR + (4 * g + j) * SVR + NOFF:QR + (4 * g + j + 1) * SVR, ts]
                     for j in range(4)], axis=1)
                ms[it] = jnp.max(jnp.maximum(mruns[it], vm), axis=0, keepdims=True)
            oc = []
            for j in range(4):
                cs = slice(j * QT, (j + 1) * QT)
                r0 = QR + (4 * g + j) * SVR
                if c == 0:
                    s = qs_ref[0, r0:r0 + C, ts]
                elif c == 1:
                    parts = [qs_ref[0, r0 + C:r0 + NOFF, ts], s_all[it % NBUF, C:2 * C - EX, cs]]
                    s = jnp.concatenate(parts if _ex_lo(g) == 0 else parts[::-1], axis=0)
                else:
                    s = s_all[it % NBUF, c * C:(c + 1) * C, cs]
                pr = jnp.exp2(s - ms[it][:, cs]).astype(bf16)
                oc.append(jnp.dot(_up(vt_p[4 * g + j, :, c * C:(c + 1) * C]), pr,
                                  preferred_element_type=f32))
            outs[it] = oc if c == 0 else [a + e for a, e in zip(outs[it], oc)]

        def finish(it):
            g, t = it // NT, it % NT
            for j, o in enumerate(outs[it]):
                inv = 1.0 / o[DH:DH + 1, :]
                ot_p[4 * g + j, :, t * QT:(t + 1) * QT] = _pk((o * inv).astype(bf16))

        def ffn_gate(c, r0=0, n=BQ):
            xn = _up(xc_p[r0 // 2:(r0 + n) // 2, :])
            gate = jnp.dot(xn, w1_v[:, c * FC:(c + 1) * FC], preferred_element_type=f32)
            hg = 0.5 * gate
            return hg * jnp.tanh(hg) + hg

        def ffn_up(c, act, r0=0, n=BQ):
            xn = _up(xc_p[r0 // 2:(r0 + n) // 2, :])
            cols = slice(c * FC, (c + 1) * FC)
            up = jnp.dot(xn, w3_v[:, cols], preferred_element_type=f32)
            h_p[r0 // 2:(r0 + n) // 2, cols] = _pk((act * up).astype(bf16))

        def ffn_down(lo, hi):
            return jax.lax.dot_general(w2_v[:, lo:hi], _up(h_p[:, lo:hi]), _NT_DIMS,
                                       preferred_element_type=f32)

        def wo_proj(t, r0=0, n=D):
            ot = _up(ot_p[:, :, t * QT:(t + 1) * QT].reshape(H * HP // 2, QT))
            return jnp.dot(_up(wot_p[r0 // 2:(r0 + n) // 2, :]), ot, preferred_element_type=f32)

        vpu_scores()
        dn = None
        nq = 0
        for i in range(NHEAD // 2 + 1):
            if i < NHEAD // 2:
                for c in (2 * i, 2 * i + 1):
                    ffn_up(c, ffn_gate(c))
            do_qk_run(nq, nq + QK_SPREAD[i])
            nq += QK_SPREAD[i]
            if i > 0:
                part = ffn_down(2 * (i - 1) * FC, 2 * i * FC)
                dn = part if dn is None else dn + part
        acc_ref[zs] = dn
        do_qk_run(nq, _PV_POS[0])

        pv = 0
        for k in range(_PV_POS[0], len(_SLOTS) + 1):
            i = 0
            while True:
                while pv < len(_FINE) and _FINE[pv] <= k * SPL + i:
                    do_pv(pv)
                    if pv % NC == NC - 1:
                        finish(pv // NC)
                    pv += 1
                if k == len(_SLOTS) or i == SPL:
                    break
                j = i + 1
                while j < SPL and not (pv < len(_FINE) and _FINE[pv] <= k * SPL + j):
                    j += 1
                do_qk(k, part=(i, j))
                i = j
                if i == SPL:
                    break

        fill = [(kind, c, i) for c in range(NHEAD, NFFN) for i in range(NT)
                for kind in ("gate", "up")]
        fill += [("wo", 0, i) for i in range(NWS)]
        accs = []
        act = None
        for c in range(TPV):
            for k, (kind, fc, i) in enumerate(fill):
                if k * TPV // len(fill) != c:
                    continue
                if kind == "gate":
                    act = ffn_gate(fc, i * QT, QT)
                elif kind == "up":
                    ffn_up(fc, act, i * QT, QT)
                else:
                    assert pv >= (NITEM - 1) * NC
                    r0, n = i * D // NWS, D // NWS
                    accs.append(acc_ref[zl, r0:r0 + n, 0:QT] + wo_proj(0, r0, n))
            do_pv(pv)
            if pv == (NITEM - 1) * NC - 1:
                finish(NITEM - 2)
            pv += 1
        acc = ffn_down(NHEAD * FC, F) + x_v[:, pl.ds(q0, BQ)].astype(f32)
        out_v[:, pl.ds(q0, QT)] = (jnp.concatenate(accs, axis=0) + acc[:, 0:QT]).astype(bf16)
        out_copy(b, 0).start()
        finish(NITEM - 1)
        acc = (acc[:, QT:BQ] + acc_ref[zl, :, QT:BQ]) + wo_proj(1)
        out_v[:, pl.ds(pl.multiple_of(q0 + QT, QT), QT)] = acc.astype(bf16)
        out_copy(b, 1).start()
        s_all[0, 0:16, 0:QT] = acc[0:16]
        return carry

    jax.lax.fori_loop(0, S // BQ, body, 0)
    for b in range(S // BQ):
        for t in range(NT):
            out_copy(b, t).wait()


@jax.jit
def pallas_parallel_sum__softmax_full_mha__glu_gated_swiglu__prompt_kernel(
    A_x: jax.Array,
    A_wqkv: jax.Array,
    A_wo: jax.Array,
    B_x: jax.Array,
    B_w1: jax.Array,
    B_w3: jax.Array,
    B_w2: jax.Array,
):
    del B_x
    xt = A_x.reshape(S, D).T
    hbm_spec = pl.BlockSpec(memory_space=pltpu.MemorySpace.HBM)
    out = pl.pallas_call(
        _kernel,
        out_shape=jax.ShapeDtypeStruct((D, S), bf16),
        in_specs=[hbm_spec] * 6,
        out_specs=hbm_spec,
        scratch_shapes=[
            pltpu.VMEM((D, S), bf16),
            pltpu.VMEM((D, 3 * D), bf16),
            pltpu.VMEM((D, D), bf16),
            pltpu.VMEM((D, F), bf16),
            pltpu.VMEM((D, F), bf16),
            pltpu.VMEM((D, F), bf16),
            pltpu.VMEM((S // 2, D), u32),
            pltpu.VMEM((BQ // 2, D), u32),
            pltpu.VMEM((3 * D // 2, D), u32),
            pltpu.VMEM((D // 2, H * HP), u32),
            pltpu.VMEM((D, TT), f32),
            pltpu.VMEM((256, TT), f32),
            pltpu.VMEM((G, S // 2, 128), u32),
            pltpu.VMEM((H, HP // 2, S), u32),
            pltpu.VMEM((1, QR + H * SVR, BQ), f32),
            pltpu.VMEM((H, HP // 2, S), u32),
            pltpu.VMEM((D, C, 128), f32),
            pltpu.VMEM((D, EX, 128), f32),
            pltpu.VMEM((H, HP // 2, BQ), u32),
            pltpu.VMEM((BQ // 2, F), u32),
            pltpu.VMEM((1, D, BQ), f32),
            pltpu.VMEM((D, S), bf16),
            pltpu.SMEM((2,), jnp.int32),
            pltpu.SemaphoreType.DMA((6,)),
            pltpu.VMEM((NBUF, S, W), f32),
        ],
        compiler_params=pltpu.CompilerParams(vmem_limit_bytes=112 * 1024 * 1024),
    )(xt, A_wqkv, A_wo, B_w1, B_w3, B_w2.T)
    return out.T.reshape(1, S, D)
```
